```python
import jax
import jax.numpy as jnp

def _softmax(x, axis=-1):
    return jax.nn.softmax(x, axis=axis)
def _gelu(x):
    return jax.nn.gelu(x, approximate=True)
def _silu(x):
    return jax.nn.silu(x)
def _sigmoid(x):
    return jax.nn.sigmoid(x)
def _layernorm(x, axis=-1, eps=1e-5):
    m = jnp.mean(x, axis=axis, keepdims=True)
    v = jnp.var(x, axis=axis, keepdims=True)
    return (x - m) / jnp.sqrt(v + eps)
def _scatter_add(tgt, idx, src, axis=0):
    return tgt.at[idx].add(src)
def _segment_sum(src, seg, n):
    return jax.ops.segment_sum(src, seg, n)
class _Rng:
    def __init__(self, key):
        self._k = key
    def _next(self):
        self._k, sub = jax.random.split(self._k)
        return sub
    def normal(self, shape):
        return jax.random.normal(self._next(), shape, dtype=jnp.bfloat16)
    def randint(self, lo, hi, shape):
        return jax.random.randint(self._next(), shape, lo, hi, dtype=jnp.int32)
    def uniform(self, shape, lo=0.0, hi=1.0):
        return jax.random.uniform(self._next(), shape, jnp.bfloat16, lo, hi)
    def permutation(self, n):
        return jax.random.permutation(self._next(), n)


kernel_name = 'interleave_layers__sliding_local_dilated__mixer_token_mlp__prompt'

def setup_inputs():
    _rng = _Rng(jax.random.key(int.from_bytes(__import__("os").urandom(4), "little")))
    _w = (lambda a: (lambda t: t.astype(jnp.bfloat16) if jnp.issubdtype(t.dtype, jnp.floating) else t)(jnp.asarray(a)))
    def _A_setup():
        B, S, D = 1, 2048, 1024
        return {
            "x": _w((lambda *s: _rng.normal(s) * 0.05)(B, S, D)),
            "wqkv": _w((lambda *s: _rng.normal(s) * 0.05)(D, 3 * D)),
            "wo": _w((lambda *s: _rng.normal(s) * 0.05)(D, D)),
        }
    _A_in = _A_setup()

    def _B_setup():
        B, S, D, F = 1, 2048, 1024, 3584
        return {
            "x": _w((lambda *s: _rng.normal(s) * 0.05)(B, S, D)),
            "w1": _w((lambda *s: _rng.normal(s) * 0.05)(S, F) * (S ** -0.5)),
            "b1": _w((lambda *s: _rng.normal(s) * 0.05)(F) * 0.02),
            "w2": _w((lambda *s: _rng.normal(s) * 0.05)(F, S) * (F ** -0.5)),
            "b2": _w((lambda *s: _rng.normal(s) * 0.05)(S) * 0.02),
        }
    _B_in = _B_setup()

    return {
        "A_x": _A_in["x"],
        "A_wqkv": _A_in["wqkv"],
        "A_wo": _A_in["wo"],
        "B_x": _B_in["x"],
        "B_w1": _B_in["w1"],
        "B_b1": _B_in["b1"],
        "B_w2": _B_in["w2"],
        "B_b2": _B_in["b2"],
    }

def reference(A_x, A_wqkv, A_wo, B_x, B_w1, B_b1, B_w2, B_b2):
    def _A_ref(x, wqkv, wo):
        B, S, D = x.shape
        H = 32; Dh = D // H
        W, dil = 8, 2
        qkv = (lambda x, *d: x.transpose(*d))((x @ wqkv).reshape(B, S, 3, H, Dh), 2, 0, 3, 1, 4)
        q, k, v = qkv[0], qkv[1], qkv[2]
        scale = Dh ** -0.5
        pos = jnp.arange(S)
        off = jnp.arange(W) * dil
        idx = pos[:, None] - off[None, :]
        mask = idx >= 0
        idx_c = jnp.where(mask, idx, 0).reshape(-1)
        kg = k[:, :, idx_c, :].reshape(B, H, S, W, Dh)
        vg = v[:, :, idx_c, :].reshape(B, H, S, W, Dh)
        logits = jnp.einsum("bhsd,bhswd->bhsw", q, kg) * scale
        logits = jnp.where(mask[None, None, :, :], logits, -1e9)
        attn = _softmax(logits, axis=-1)
        o = jnp.einsum("bhsw,bhswd->bhsd", attn, vg)
        return (lambda x, *d: x.transpose(*d))(o, 0, 2, 1, 3).reshape(B, S, D) @ wo

    def _B_ref(x, w1, b1, w2, b2):
        B, S, D = x.shape
        h = _layernorm(x, axis=-1)
        u = jnp.einsum("bsd,sf->bdf", h, w1) + b1
        u = _gelu(u)
        y = jnp.einsum("bdf,fs->bds", u, w2) + b2
        return (lambda x, *d: x.transpose(*d))(y, 0, 2, 1)

    x = A_x
    x = x + _A_ref(_layernorm(x, axis=-1), A_wqkv, A_wo)
    x = x + _B_ref(_layernorm(x, axis=-1), B_w1, B_b1, B_w2, B_b2)
    x = x + _A_ref(_layernorm(x, axis=-1), A_wqkv, A_wo)
    x = x + _B_ref(_layernorm(x, axis=-1), B_w1, B_b1, B_w2, B_b2)
    return x
```

```python
import functools
import math

import jax
import jax.numpy as jnp
from jax import lax
import jax.experimental.pallas as pl
import jax.experimental.pallas.tpu as pltpu

S = 2048
D = 1024
F = 3584
H = 32
DH = D // H
W = 8
DIL = 2
HALO = 16
EPS = 1e-5
TM = 256
NCH = S // TM
TB = 256
NB = D // TB
NT = D // 128
RG = 8
BF16 = jnp.bfloat16
F32 = jnp.float32
EXP2_SCALE = (DH ** -0.5) * math.log2(math.e)
GELU_C = math.sqrt(2.0 / math.pi)


def _permute_cols(w):
    u = pltpu.bitcast(w, jnp.uint32)
    tiles = [u[:, j * 128:(j + 1) * 128] for j in range(NT)]
    lane = lax.broadcasted_iota(jnp.int32, tiles[0].shape, 1)
    for tb, lb in ((2, 4), (1, 3), (0, 2)):
        keep = ((lane >> lb) & 1) == 0
        new = list(tiles)
        for j in range(NT):
            if (j >> tb) & 1:
                continue
            a, b = tiles[j], tiles[j | (1 << tb)]
            new[j] = jnp.where(keep, a, pltpu.roll(b, 1 << lb, 1))
            new[j | (1 << tb)] = jnp.where(keep, pltpu.roll(a, 128 - (1 << lb), 1), b)
        tiles = new
    return pltpu.bitcast(jnp.concatenate(tiles, axis=1), BF16)


def _ln_stats(x):
    m = jnp.sum(x, axis=0, keepdims=True) * (1.0 / D)
    xc = x - m
    v = jnp.sum(xc * xc, axis=0, keepdims=True) * (1.0 / D)
    return xc, v


def _kernel(x_hbm, wqkv_hbm, wo_hbm, w1_hbm, b1_ref, w2_hbm, b2_ref, out_hbm,
            xt, ht, wqkv, wot, w1, w2, xin, xn0, xn1,
            q0, k0, v0, q1, k1, v1, sbuf, obuf, stage, sem_in, sem_out):
    xn = (xn0, xn1)
    qb, kb, vb = (q0, q1), (k0, k1), (v0, v1)

    cp_x = [pltpu.make_async_copy(x_hbm.at[pl.ds(c * TM, TM), :], xin.at[c], sem_in.at[c])
            for c in range(NCH)]
    NWP = 8
    RW = D // NWP
    cp_wqkv = [pltpu.make_async_copy(wqkv_hbm.at[pl.ds(i * RW, RW), :], wqkv.at[pl.ds(i * RW, RW), :],
                                     sem_in.at[NCH + i]) for i in range(NWP)]
    cp_wo = pltpu.make_async_copy(wo_hbm, wot, sem_in.at[NCH + NWP])
    cp_w1 = pltpu.make_async_copy(w1_hbm, w1, sem_in.at[NCH + NWP + 1])
    cp_w2 = pltpu.make_async_copy(w2_hbm, w2, sem_in.at[NCH + NWP + 2])
    for cp in cp_wqkv[:2]:
        cp.start()
    cp_x[0].start()
    for cp in cp_wqkv[2:]:
        cp.start()
    for cp in cp_x[1:]:
        cp.start()
    cp_wo.start()

    for i in range(NWP):
        cp_wqkv[i].wait()
        rows = pl.ds(i * RW, RW)
        for t in range(3):
            wqkv[rows, t * D:(t + 1) * D] = _permute_cols(wqkv[rows, t * D:(t + 1) * D])
    cp_w1.start()
    cp_w2.start()
    for c in range(NCH):
        cp_x[c].wait()
        xt[c] = xin[c].astype(F32).T
    cp_wo.wait()
    wo_t = wot[...].T
    for i in range(NWP):
        wot[i * RW:(i + 1) * RW, :] = _permute_cols(wo_t[i * RW:(i + 1) * RW, :])

    for b in (k1, v1):
        b[:, TM:TM + HALO, :] = jnp.zeros((NT, HALO, 128), F32)
    for b in (k0, v0):
        b[:, TM:TM + HALO, :] = jnp.zeros((NT, HALO, 128), F32)

    li = lax.broadcasted_iota(jnp.int32, (128, 128), 0) >> 2
    lj = lax.broadcasted_iota(jnp.int32, (128, 128), 1) >> 2
    rsum = (li == lj).astype(BF16)

    def stage_p(c, p):
        xc, v = _ln_stats(xt[c])
        y = (xc * lax.rsqrt(v + EPS)).astype(BF16)
        xn[p][...] = y.T

    def stage_q(p_x, p, t0, t1, first):
        res = jnp.dot(xn[p_x][...], wqkv[:, t0 * 128:t1 * 128], preferred_element_type=F32)
        for t in range(t0, t1):
            piece = res[:, (t - t0) * 128:(t - t0 + 1) * 128]
            kind, j = divmod(t, NT)
            if kind == 0:
                qb[p][j] = piece
            else:
                dst = (kb if kind == 1 else vb)[p]
                src = (kb if kind == 1 else vb)[1 - p]
                if first:
                    dst[j, 0:HALO, :] = jnp.zeros((HALO, 128), F32)
                else:
                    dst[j, 0:HALO, :] = src[j, TM:TM + HALO, :]
                dst[j, HALO:HALO + TM, :] = piece

    def stage_s1(p, r0, r1):
        for r in range(r0, r1, RG):
            q = [qb[p][j, r:r + RG, :] for j in range(NT)]
            for w in range(W):
                o = HALO - DIL * w + r
                acc = q[0] * kb[p][0, o:o + RG, :]
                for j in range(1, NT):
                    acc = acc + q[j] * kb[p][j, o:o + RG, :]
                sbuf[w, r:r + RG, :] = acc

    def stage_r(r0, r1):
        s = jnp.concatenate([sbuf[w, r0:r1, :].astype(BF16) for w in range(W)], axis=0)
        lg = jnp.dot(s, rsum, preferred_element_type=F32)
        n = r1 - r0
        return [lg[w * n:(w + 1) * n] for w in range(W)]

    def stage_s3(c, p, lg, r0, r1):
        for r in range(r0, r1, RG):
            s = [lg[w][r - r0:r - r0 + RG] for w in range(W)]
            if r < HALO:
                row = c * TM + r + lax.broadcasted_iota(jnp.int32, (RG, 128), 0)
                s = [s[0]] + [jnp.where(row >= DIL * w, s[w], -1e30) for w in range(1, W)]
            m = s[0]
            for w in range(1, W):
                m = jnp.maximum(m, s[w])
            e = [jnp.exp2((s[w] - m) * EXP2_SCALE) for w in range(W)]
            l = e[0]
            for w in range(1, W):
                l = l + e[w]
            inv = 1.0 / l
            outs = []
            for j in range(NT):
                acc = e[0] * vb[p][j, HALO + r:HALO + r + RG, :]
                for w in range(1, W):
                    o = HALO - DIL * w + r
                    acc = acc + e[w] * vb[p][j, o:o + RG, :]
                outs.append(acc * inv)
            obuf[r:r + RG, :] = jnp.concatenate(outs, axis=1)

    def stage_o():
        return lax.dot_general(wot[...], obuf[...].astype(BF16), (((1,), (1,)), ((), ())),
                               preferred_element_type=F32)

    def stage_e(c, out_t):
        x = xt[c] + out_t
        xt[c] = x
        xc, v = _ln_stats(x)
        r1 = lax.rsqrt(v + EPS)
        r2 = lax.rsqrt(v * r1 * r1 + EPS)
        ht[c] = (xc * (r1 * r2)).astype(BF16)

    def step(c, p, do_p, do_q):
        if do_p:
            stage_p(c + 2, p)
        if do_q:
            stage_q(1 - p, 1 - p, 0, 8, False)
        stage_s1(p, 0, TM)
        lg = stage_r(0, TM)
        if do_q:
            stage_q(1 - p, 1 - p, 8, 16, False)
        stage_s3(c, p, lg, 0, TM)
        out_t = stage_o()
        if do_q:
            stage_q(1 - p, 1 - p, 16, 24, False)
        stage_e(c, out_t)

    def phase_a():
        stage_p(0, 0)
        stage_p(1, 1)
        stage_q(0, 0, 0, 24, True)

        def body(k, carry):
            step(2 * k, 0, True, True)
            step(2 * k + 1, 1, True, True)
            return carry
        lax.fori_loop(0, NCH // 2 - 1, body, 0)
        step(NCH - 2, 0, False, True)
        step(NCH - 1, 1, False, False)

    def out_copy(m):
        return pltpu.make_async_copy(stage.at[m], out_hbm.at[:, pl.ds(m * TB, TB)], sem_out.at[m])

    def phase_b(l):
        b1 = b1_ref[...].astype(F32)
        b2 = b2_ref[...].astype(F32)

        def body(m, carry):
            rows = pl.ds(pl.multiple_of(m * TB, TB), TB)
            lhs = jnp.concatenate([ht[c, rows, :] for c in range(NCH)], axis=1)
            u = jnp.dot(lhs, w1[...], preferred_element_type=F32) + b1
            u = 0.5 * u * (1.0 + jnp.tanh(GELU_C * (u + 0.044715 * (u * u * u))))
            y = jnp.dot(u.astype(BF16), w2[...], preferred_element_type=F32) + b2
            for c in range(NCH):
                xnew = xt[c, rows, :] + y[:, c * TM:(c + 1) * TM]
                xt[c, rows, :] = xnew
                stage[m, c * TM:(c + 1) * TM, :] = xnew.astype(BF16).T

            @pl.when(l == 1)
            def _():
                pltpu.make_async_copy(stage.at[m], out_hbm.at[:, pl.ds(pl.multiple_of(m * TB, TB), TB)],
                                      sem_out.at[m]).start()
            return carry
        lax.fori_loop(0, NB, body, 0)

    def layer(l, carry):
        phase_a()

        @pl.when(l == 0)
        def _():
            cp_w1.wait()
            cp_w2.wait()
        phase_b(l)
        return carry
    lax.fori_loop(0, 2, layer, 0)
    for m in range(NB):
        out_copy(m).wait()


@jax.jit
def pallas_interleave_layers__sliding_local_dilated__mixer_token_mlp__prompt_kernel(
    A_x: jax.Array,
    A_wqkv: jax.Array,
    A_wo: jax.Array,
    B_x: jax.Array,
    B_w1: jax.Array,
    B_b1: jax.Array,
    B_w2: jax.Array,
    B_b2: jax.Array,
):
    del B_x
    x = A_x.reshape(S, D)
    any_spec = pl.BlockSpec(memory_space=pl.ANY)
    vmem_spec = pl.BlockSpec(memory_space=pltpu.VMEM)
    scratch = [
        pltpu.VMEM((NCH, D, TM), F32),
        pltpu.VMEM((NCH, D, TM), BF16),
        pltpu.VMEM((D, 3 * D), BF16),
        pltpu.VMEM((D, D), BF16),
        pltpu.VMEM((S, F), BF16),
        pltpu.VMEM((F, S), BF16),
        pltpu.VMEM((NCH, TM, D), BF16),
        pltpu.VMEM((TM, D), BF16),
        pltpu.VMEM((TM, D), BF16),
        pltpu.VMEM((NT, TM, 128), F32),
        pltpu.VMEM((NT, TM + HALO, 128), F32),
        pltpu.VMEM((NT, TM + HALO, 128), F32),
        pltpu.VMEM((NT, TM, 128), F32),
        pltpu.VMEM((NT, TM + HALO, 128), F32),
        pltpu.VMEM((NT, TM + HALO, 128), F32),
        pltpu.VMEM((W, TM, 128), F32),
        pltpu.VMEM((TM, D), F32),
        pltpu.VMEM((NB, S, TB), BF16),
        pltpu.SemaphoreType.DMA((NCH + 8 + 3,)),
        pltpu.SemaphoreType.DMA((NB,)),
    ]
    out = pl.pallas_call(
        _kernel,
        out_shape=jax.ShapeDtypeStruct((S, D), BF16),
        in_specs=[any_spec, any_spec, any_spec, any_spec, vmem_spec, any_spec, vmem_spec],
        out_specs=any_spec,
        scratch_shapes=scratch,
        compiler_params=pltpu.CompilerParams(vmem_limit_bytes=110 * 1024 * 1024),
    )(x, A_wqkv, A_wo, B_w1, B_b1.reshape(1, F), B_w2, B_b2.reshape(1, S))
    return out.reshape(1, S, D)
```

```python
import functools
import math
import os

import jax
import jax.numpy as jnp
from jax import lax
import jax.experimental.pallas as pl
import jax.experimental.pallas.tpu as pltpu

S = 2048
D = 1024
F = 3584
H = 32
DH = D // H
W = 8
DIL = 2
HALO = 16
EPS = 1e-5
TM = 256
NCH = S // TM
TB = int(os.environ.get('TB', '128'))
NB = D // TB
NT = D // 128
RG = 8
RB = 64
NSLOT = S // RB
SB = int(os.environ.get("SB", "32"))
PINS = os.environ.get("PINS", "none").split(",")
GCH = int(os.environ.get("GCH", "0"))
JOUT = int(os.environ.get("JOUT", "0"))
RCP = int(os.environ.get("RCP", "0"))
XU = int(os.environ.get("XU", "1"))
NRUN = int(os.environ.get("NRUN", "8"))
ONLY_A = int(os.environ.get("ONLY_A", "0"))
SKIP = os.environ.get('SKIP', '').split(',')
BF16 = jnp.bfloat16
F32 = jnp.float32
U32 = jnp.uint32
I32 = jnp.int32
EXP2_SCALE = (DH ** -0.5) * math.log2(math.e)
GELU_C = math.sqrt(2.0 / math.pi)


def _permute_cols_u32(w):
    u = pltpu.bitcast(w, U32)
    tiles = [u[:, j * 128:(j + 1) * 128] for j in range(NT)]
    lane = lax.broadcasted_iota(I32, tiles[0].shape, 1)
    for tb, lb in ((2, 4), (1, 3), (0, 2)):
        keep = ((lane >> lb) & 1) == 0
        new = list(tiles)
        for j in range(NT):
            if (j >> tb) & 1:
                continue
            a, b = tiles[j], tiles[j | (1 << tb)]
            new[j] = jnp.where(keep, a, pltpu.roll(b, 1 << lb, 1))
            new[j | (1 << tb)] = jnp.where(keep, pltpu.roll(a, 128 - (1 << lb), 1), b)
        tiles = new
    return jnp.concatenate(tiles, axis=1)


def _ln_stats(x):
    m = jnp.sum(x, axis=0, keepdims=True) * (1.0 / D)
    xc = x - m
    v = jnp.sum(xc * xc, axis=0, keepdims=True) * (1.0 / D)
    return xc, v


def _ortree(x):
    u = x if x.dtype == U32 else pltpu.bitcast(x, U32)
    r, c = u.shape
    acc = None
    for i in range(r // 8):
        for j in range(c // 128):
            blk = u[i * 8:(i + 1) * 8, j * 128:(j + 1) * 128]
            acc = blk if acc is None else (acc | blk)
    return acc


def _kernel(zero_ref, x_hbm, wqkv_hbm, wo_hbm, w1_hbm, b1_ref, w2_hbm, b2_ref, out_hbm,
            xt, ht, wraw, wqkv, wot, w1, w2, xin, xn, qb, kb, vb, obuf, stage, sem_in, sem_out):
    cp_x = [pltpu.make_async_copy(x_hbm.at[pl.ds(c * TM, TM), :], xin.at[c], sem_in.at[c])
            for c in range(NCH)]
    cp_w = [pltpu.make_async_copy(wqkv_hbm.at[:, pl.ds(t * D, D)], wraw.at[t], sem_in.at[NCH + t]) for t in range(3)]
    cp_w.append(pltpu.make_async_copy(wo_hbm, wraw.at[3], sem_in.at[NCH + 3]))
    cp_w1 = pltpu.make_async_copy(w1_hbm, w1, sem_in.at[NCH + 4])
    cp_w2 = pltpu.make_async_copy(w2_hbm, w2, sem_in.at[NCH + 5])
    for cp in (cp_x[0], cp_w[0], cp_x[1], cp_w[1], cp_w[2], cp_w[3], *cp_x[2:], cp_w1, cp_w2):
        cp.start()
    for b in (kb, vb):
        b[:, 0:HALO, :] = jnp.zeros((NT, HALO, 128), F32)

    NWP = 8
    RW = D // NWP

    def prep_w(t):
        for i in range(NWP):
            wqkv[i * RW // 2:(i + 1) * RW // 2, t * D:(t + 1) * D] = _permute_cols_u32(wraw[t, i * RW:(i + 1) * RW, :])

    def prep_wo():
        wo_t = wraw[3].T
        for i in range(NWP):
            wot[i * RW // 2:(i + 1) * RW // 2, :] = _permute_cols_u32(wo_t[i * RW:(i + 1) * RW, :])

    def load_x(c):
        xt[c] = xin[c].astype(F32).T

    zero = zero_ref[0].astype(U32)

    def pin(lhs, toks):
        toks = [t for t in toks if t is not None]
        if not toks:
            return lhs
        t = toks[0]
        for x in toks[1:]:
            t = t | x
        blk = lhs[0:8, 0:128] | (t & zero)
        top = jnp.concatenate([blk, lhs[0:8, 128:]], axis=1)
        return jnp.concatenate([top, lhs[8:]], axis=0)

    def fdep(x, tok):
        t = pltpu.bitcast(tok, U32) & zero
        return pltpu.bitcast(pltpu.bitcast(x, U32) | t, F32)

    def make_rsum():
        li = lax.broadcasted_iota(I32, (128, 128), 0) >> 2
        lj = lax.broadcasted_iota(I32, (128, 128), 1) >> 2
        return (li == lj).astype(BF16)

    def stage_p(c, h):
        if 'P' in SKIP:
            return None
        xc, v = _ln_stats(xt[c, :, h * 128:(h + 1) * 128])
        y = (xc * lax.rsqrt(v + EPS)).astype(BF16)
        u = pltpu.bitcast(y.T, U32)
        xn[c, h * 64:(h + 1) * 64, :] = u
        return _ortree(u) if 'p' in PINS else None

    def stage_q(c, t0, t1, toks):
        lhs = pltpu.bitcast(pin(xn[c], toks), BF16)
        rhs = pltpu.bitcast(wqkv[:, t0 * 128:t1 * 128], BF16)
        res = jnp.dot(lhs, rhs, preferred_element_type=F32)
        for t in range(t0, t1):
            piece = res[:, (t - t0) * 128:(t - t0 + 1) * 128]
            kind, j = divmod(t, NT)
            if kind == 0:
                qb[j, c * TM:(c + 1) * TM, :] = piece
            else:
                (kb if kind == 1 else vb)[j, HALO + c * TM:HALO + (c + 1) * TM, :] = piece

    def stage_s1(r0):
        parts = []
        tok = None
        for r in range(r0, r0 + SB, RG):
            if JOUT:
                accs = [None] * W
                for j in range(NT):
                    qj = qb[j, r:r + RG, :]
                    if GCH and tok is not None and j == 0:
                        qj = fdep(qj, tok)
                    for w in range(W):
                        o = HALO - DIL * w + r
                        t = qj * kb[j, o:o + RG, :]
                        accs[w] = t if accs[w] is None else accs[w] + t
                parts.extend(accs)
                tok = accs[W - 1]
            else:
                q = [qb[j, r:r + RG, :] for j in range(NT)]
                if GCH and tok is not None:
                    q[0] = fdep(q[0], tok)
                for w in range(W):
                    o = HALO - DIL * w + r
                    acc = q[0] * kb[0, o:o + RG, :]
                    for j in range(1, NT):
                        acc = acc + q[j] * kb[j, o:o + RG, :]
                    parts.append(acc)
                tok = parts[-1]
        s = jnp.concatenate(parts, axis=0).astype(BF16)
        return s, (_ortree(pltpu.bitcast(s, U32)) if 's1' in PINS else None)

    def stage_s3(r0, lg):
        tok = None
        res = []
        for gi, r in enumerate(range(r0, r0 + SB, RG)):
            s = [lg[(gi * W + w) * RG:(gi * W + w + 1) * RG] for w in range(W)]
            if r < HALO:
                row = r + lax.broadcasted_iota(I32, (RG, 128), 0)
                s = [s[0]] + [jnp.where(row >= DIL * w, s[w], -1e30) for w in range(1, W)]
            m = s[0]
            if GCH and res:
                m = fdep(m, res[-1][:, (NT - 1) * 128:])
            for w in range(1, W):
                m = jnp.maximum(m, s[w])
            e = [jnp.exp2((s[w] - m) * EXP2_SCALE) for w in range(W)]
            l = e[0]
            for w in range(1, W):
                l = l + e[w]
            if RCP:
                inv = pl.reciprocal(l, approx=True)
                inv = inv * (2.0 - l * inv)
            else:
                inv = 1.0 / l
            outs = []
            for j in range(NT):
                acc = e[0] * vb[j, HALO + r:HALO + r + RG, :]
                for w in range(1, W):
                    o = HALO - DIL * w + r
                    acc = acc + e[w] * vb[j, o:o + RG, :]
                outs.append(acc * inv)
            res.append(jnp.concatenate(outs, axis=1))
        o = pltpu.bitcast(jnp.concatenate(res, axis=0).astype(BF16), U32)
        obuf[r0 // 2:(r0 + SB) // 2, :] = o
        return _ortree(o) if 's3' in PINS else None

    def stage_o(n, h, toks):
        lhs = pltpu.bitcast(pin(wot[h * (D // 4):(h + 1) * (D // 4), :], toks), BF16)
        o = pltpu.bitcast(obuf[n * 64:(n + 1) * 64, :], BF16)
        return lax.dot_general(lhs, o, (((1,), (1,)), ((), ())), preferred_element_type=F32)

    def stage_e(n, out_t):
        c, hh = divmod(n, TM // 128)
        cols = slice(hh * 128, (hh + 1) * 128)
        if 'E' in SKIP:
            xt[c, :, cols] = out_t
            return None
        x = xt[c, :, cols] + out_t
        xt[c, :, cols] = x
        xc, v = _ln_stats(x)
        r1 = lax.rsqrt(v + EPS)
        r2 = lax.rsqrt(v * r1 * r1 + EPS)
        hv = (xc * (r1 * r2)).astype(BF16)
        ht[c, :, cols] = hv
        return _ortree(pltpu.bitcast(hv, U32)) if 'e' in PINS else None

    def phase_a(first):
        rsum = make_rsum()
        nslot = NRUN * (TM // RB)
        SPC = TM // RB
        NSUB = RB // SB
        if first:
            cp_x[0].wait()
            load_x(0)
            for h in range(2):
                stage_p(0, h)
            cp_w[0].wait()
            prep_w(0)
            cp_x[1].wait()
            cp_w[1].wait()
            load_x(1)
            for h in range(2):
                stage_p(1, h)
            stage_q(0, 0, 8, [])
            prep_w(1)
            cp_w[2].wait()
            stage_q(0, 8, 16, [])
            prep_w(2)
            cp_w[3].wait()
            for c in range(2, NCH):
                cp_x[c].wait()
            stage_q(0, 16, 24, [])
            prep_wo()
            load_x(2)
        else:
            for h in range(2):
                stage_p(0, h)
            for h in range(2):
                stage_p(1, h)
            stage_q(0, 0, 24, [])
        lg_prev = None
        ohalf = {}
        ptok = {}
        carry = []
        for s in range(nslot + 4):
            c, i = divmod(s, SPC)
            do_q = (c + 1 < NRUN) and s < nslot
            s3_toks = []
            if lg_prev is not None and 'ATT' not in SKIP:
                for u in range(NSUB):
                    s3_toks.append(stage_s3((s - 1) * RB + u * SB, lg_prev[u * SB * W:(u + 1) * SB * W]))
            lg_prev = None
            e_tok = None
            if s >= 5 and (s - 5) % 2 == 0 and (s - 5) // 2 < nslot // 2:
                n = (s - 5) // 2
                e_tok = stage_e(n, jnp.concatenate([ohalf.pop((n, 0)), ohalf.pop((n, 1))], axis=0))
            p_tok = None
            if first and i == 0 and c + 3 < NRUN:
                load_x(c + 3)
            if c + 2 < NRUN and i % 2 == 1 and s < nslot:
                p_tok = stage_p(c + 2, i // 2)
            s1 = []
            if s < nslot and 'ATT' not in SKIP:
                s1 = [stage_s1(s * RB + u * SB) for u in range(NSUB)]
            half = max(1, NSUB // 2)
            pins1 = carry
            pins2 = s3_toks[:half]
            pinso = s3_toks[half:]
            pins3 = [e_tok] + [t for _, t in s1[:half]]
            carry = [p_tok]
            t0 = 6 * i
            qs = [int(x) for x in os.environ.get("QS", "2,2,2").split(",")]
            opos = int(os.environ.get("OPOS", "2"))
            allp = [pins1, pins2, pins3]
            tt = t0
            for qi, qn in enumerate(qs + [0]):
                if qi == opos and s >= 3 and (s - 3) // 2 < nslot // 2:
                    n, h = divmod(s - 3, 2)
                    ohalf[(n, h)] = stage_o(n, h, pinso if do_q else [])
                if do_q and qn:
                    if len(qs) == 3:
                        pp = allp[qi]
                    elif len(qs) == 2:
                        pp = [pins1, pins2 + pins3][qi]
                    else:
                        pp = pins1
                    stage_q(c + 1, tt, tt + qn, pp)
                tt += qn
            if s1:
                sc = jnp.concatenate([x for x, _ in s1], axis=0)
                lg_prev = jnp.dot(sc, rsum, preferred_element_type=F32)

    def phase_b(l):
        b1 = b1_ref[...].astype(F32)
        b2 = b2_ref[...].astype(F32)
        def body(m, carry):
            with jax.named_scope("b_iter"):
                rows = pl.ds(pl.multiple_of(m * TB, TB), TB)
                lhs = jnp.concatenate([ht[c, rows, :] for c in range(NCH)], axis=1)
                u = jnp.dot(lhs, w1[...], preferred_element_type=F32) + b1
                u = 0.5 * u * (1.0 + jnp.tanh(GELU_C * (u + 0.044715 * (u * u * u))))
                y = jnp.dot(u.astype(BF16), w2[...], preferred_element_type=F32) + b2
                for c in range(NCH):
                    xnew = xt[c, rows, :] + y[:, c * TM:(c + 1) * TM]
                    if l == 0:
                        xt[c, rows, :] = xnew
                    else:
                        stage[m, c * TM:(c + 1) * TM, :] = xnew.astype(BF16).T

                if l == 1:
                    pltpu.make_async_copy(stage.at[m], out_hbm.at[:, pl.ds(pl.multiple_of(m * TB, TB), TB)],
                                          sem_out.at[m]).start()
            return carry
        lax.fori_loop(0, NB, body, 0)

    def out_copy(m):
        return pltpu.make_async_copy(stage.at[m], out_hbm.at[:, pl.ds(m * TB, TB)], sem_out.at[m])

    for l in range(2):
        with jax.named_scope("phase_a"):
            phase_a(l == 0)
        if l == 0:
            cp_w1.wait()
            cp_w2.wait()
        if not ONLY_A:
            with jax.named_scope("phase_b"):
                phase_b(l)
    if ONLY_A:
        for m in range(NB):
            stage[m] = jnp.zeros((S, TB), BF16)
        stage[0, 0:TM, :] = ht[0, 0:TB, :]
    if ONLY_A:
        for m in range(NB):
            out_copy(m).start()
    for m in range(NB):
        out_copy(m).wait()


@jax.jit
def pallas_interleave_layers__sliding_local_dilated__mixer_token_mlp__prompt_kernel(
    A_x, A_wqkv, A_wo, B_x, B_w1, B_b1, B_w2, B_b2):
    del B_x
    x = A_x.reshape(S, D)
    any_spec = pl.BlockSpec(memory_space=pl.ANY)
    vmem_spec = pl.BlockSpec(memory_space=pltpu.VMEM)
    smem_spec = pl.BlockSpec(memory_space=pltpu.SMEM)
    scratch = [
        pltpu.VMEM((NCH, D, TM), F32),
        pltpu.VMEM((NCH, D, TM), BF16),
        pltpu.VMEM((4, D, D), BF16),
        pltpu.VMEM((D // 2, 3 * D), U32),
        pltpu.VMEM((D // 2, D), U32),
        pltpu.VMEM((S, F), BF16),
        pltpu.VMEM((F, S), BF16),
        pltpu.VMEM((NCH, TM, D), BF16),
        pltpu.VMEM((NCH, TM // 2, D), U32),
        pltpu.VMEM((NT, S, 128), F32),
        pltpu.VMEM((NT, S + HALO, 128), F32),
        pltpu.VMEM((NT, S + HALO, 128), F32),
        pltpu.VMEM((S // 2, D), U32),
        pltpu.VMEM((NB, S, TB), BF16),
        pltpu.SemaphoreType.DMA((NCH + 6,)),
        pltpu.SemaphoreType.DMA((NB,)),
    ]
    out = pl.pallas_call(
        _kernel,
        out_shape=jax.ShapeDtypeStruct((S, D), BF16),
        in_specs=[smem_spec, any_spec, any_spec, any_spec, any_spec, vmem_spec, any_spec, vmem_spec],
        out_specs=any_spec,
        scratch_shapes=scratch,
        compiler_params=pltpu.CompilerParams(vmem_limit_bytes=124 * 1024 * 1024),
    )(jnp.zeros((1,), jnp.int32), x, A_wqkv, A_wo, B_w1, B_b1.reshape(1, F), B_w2, B_b2.reshape(1, S))
    return out.reshape(1, S, D)
```

```python
import functools
import math
import os

import jax
import jax.numpy as jnp
from jax import lax
import jax.experimental.pallas as pl
import jax.experimental.pallas.tpu as pltpu

S = 2048
D = 1024
F = 3584
H = 32
DH = D // H
W = 8
DIL = 2
HALO = 16
EPS = 1e-5
TM = 256
NCH = S // TM
TB = int(os.environ.get('TB', '128'))
NB = D // TB
NT = D // 128
RG = 8
RB = 64
NSLOT = S // RB
SB = int(os.environ.get("SB", "32"))
PINS = os.environ.get("PINS", "none").split(",")
GCH = int(os.environ.get("GCH", "0"))
JOUT = int(os.environ.get("JOUT", "0"))
RCP = int(os.environ.get("RCP", "0"))
XU = int(os.environ.get("XU", "1"))
NRUN = int(os.environ.get("NRUN", "8"))
ONLY_A = int(os.environ.get("ONLY_A", "0"))
SKIP = os.environ.get('SKIP', '').split(',')
BF16 = jnp.bfloat16
F32 = jnp.float32
U32 = jnp.uint32
I32 = jnp.int32
EXP2_SCALE = (DH ** -0.5) * math.log2(math.e)
GELU_C = math.sqrt(2.0 / math.pi)


def _permute_cols_u32(w):
    u = pltpu.bitcast(w, U32)
    tiles = [u[:, j * 128:(j + 1) * 128] for j in range(NT)]
    lane = lax.broadcasted_iota(I32, tiles[0].shape, 1)
    for tb, lb in ((2, 4), (1, 3), (0, 2)):
        keep = ((lane >> lb) & 1) == 0
        new = list(tiles)
        for j in range(NT):
            if (j >> tb) & 1:
                continue
            a, b = tiles[j], tiles[j | (1 << tb)]
            new[j] = jnp.where(keep, a, pltpu.roll(b, 1 << lb, 1))
            new[j | (1 << tb)] = jnp.where(keep, pltpu.roll(a, 128 - (1 << lb), 1), b)
        tiles = new
    return jnp.concatenate(tiles, axis=1)


def _ln_stats(x):
    m = jnp.sum(x, axis=0, keepdims=True) * (1.0 / D)
    xc = x - m
    v = jnp.sum(xc * xc, axis=0, keepdims=True) * (1.0 / D)
    return xc, v


def _ortree(x):
    u = x if x.dtype == U32 else pltpu.bitcast(x, U32)
    r, c = u.shape
    acc = None
    for i in range(r // 8):
        for j in range(c // 128):
            blk = u[i * 8:(i + 1) * 8, j * 128:(j + 1) * 128]
            acc = blk if acc is None else (acc | blk)
    return acc


def _kernel(zero_ref, x_hbm, wqkv_hbm, wo_hbm, w1_hbm, b1_ref, w2_hbm, b2_ref, out_hbm,
            xt, ht, wraw, wqkv, wot, w1, w2, xin, xn, qb, kb, vb, obuf, stage, sem_in, sem_out):
    cp_x = [pltpu.make_async_copy(x_hbm.at[pl.ds(c * TM, TM), :], xin.at[c], sem_in.at[c])
            for c in range(NCH)]
    NQP = 4
    cp_wq = [pltpu.make_async_copy(wqkv_hbm.at[pl.ds(i * (D // NQP), D // NQP), pl.ds(0, D)],
                                   wraw.at[0, pl.ds(i * (D // NQP), D // NQP), :], sem_in.at[NCH + 6 + i])
             for i in range(NQP)]
    cp_w = [None] + [pltpu.make_async_copy(wqkv_hbm.at[:, pl.ds(t * D, D)], wraw.at[t], sem_in.at[NCH + t])
                     for t in range(1, 3)]
    cp_w.append(pltpu.make_async_copy(wo_hbm, wraw.at[3], sem_in.at[NCH + 3]))
    cp_w1 = pltpu.make_async_copy(w1_hbm, w1, sem_in.at[NCH + 4])
    cp_w2 = pltpu.make_async_copy(w2_hbm, w2, sem_in.at[NCH + 5])
    for cp in (cp_x[0], *cp_wq, cp_x[1], cp_w[1]):
        cp.start()
    for b in (kb, vb):
        b[:, 0:HALO, :] = jnp.zeros((NT, HALO, 128), F32)

    NWP = 8
    RW = D // NWP

    def prep_w(t, i0=0, i1=8):
        for i in range(i0, i1):
            wqkv[i * RW // 2:(i + 1) * RW // 2, t * D:(t + 1) * D] = _permute_cols_u32(wraw[t, i * RW:(i + 1) * RW, :])

    def prep_wo():
        wo_t = wraw[3].T
        for i in range(NWP):
            wot[i * RW // 2:(i + 1) * RW // 2, :] = _permute_cols_u32(wo_t[i * RW:(i + 1) * RW, :])

    def load_x(c):
        xt[c] = xin[c].astype(F32).T

    zero = zero_ref[0].astype(U32)

    def pin(lhs, toks):
        toks = [t for t in toks if t is not None]
        if not toks:
            return lhs
        t = toks[0]
        for x in toks[1:]:
            t = t | x
        blk = lhs[0:8, 0:128] | (t & zero)
        top = jnp.concatenate([blk, lhs[0:8, 128:]], axis=1)
        return jnp.concatenate([top, lhs[8:]], axis=0)

    def fdep(x, tok):
        t = pltpu.bitcast(tok, U32) & zero
        return pltpu.bitcast(pltpu.bitcast(x, U32) | t, F32)

    def make_rsum():
        li = lax.broadcasted_iota(I32, (128, 128), 0) >> 2
        lj = lax.broadcasted_iota(I32, (128, 128), 1) >> 2
        return (li == lj).astype(BF16)

    def stage_p(c, h):
        if 'P' in SKIP:
            return None
        xc, v = _ln_stats(xt[c, :, h * 128:(h + 1) * 128])
        y = (xc * lax.rsqrt(v + EPS)).astype(BF16)
        u = pltpu.bitcast(y.T, U32)
        xn[c, h * 64:(h + 1) * 64, :] = u
        return _ortree(u) if 'p' in PINS else None

    def stage_q(c, t0, t1, toks):
        lhs = pltpu.bitcast(pin(xn[c], toks), BF16)
        rhs = pltpu.bitcast(wqkv[:, t0 * 128:t1 * 128], BF16)
        res = jnp.dot(lhs, rhs, preferred_element_type=F32)
        for t in range(t0, t1):
            piece = res[:, (t - t0) * 128:(t - t0 + 1) * 128]
            kind, j = divmod(t, NT)
            if kind == 0:
                qb[j, c * TM:(c + 1) * TM, :] = piece
            else:
                (kb if kind == 1 else vb)[j, HALO + c * TM:HALO + (c + 1) * TM, :] = piece

    def stage_s1(r0):
        parts = []
        tok = None
        for r in range(r0, r0 + SB, RG):
            if JOUT:
                accs = [None] * W
                for j in range(NT):
                    qj = qb[j, r:r + RG, :]
                    if GCH and tok is not None and j == 0:
                        qj = fdep(qj, tok)
                    for w in range(W):
                        o = HALO - DIL * w + r
                        t = qj * kb[j, o:o + RG, :]
                        accs[w] = t if accs[w] is None else accs[w] + t
                parts.extend(accs)
                tok = accs[W - 1]
            else:
                q = [qb[j, r:r + RG, :] for j in range(NT)]
                if GCH and tok is not None:
                    q[0] = fdep(q[0], tok)
                for w in range(W):
                    o = HALO - DIL * w + r
                    acc = q[0] * kb[0, o:o + RG, :]
                    for j in range(1, NT):
                        acc = acc + q[j] * kb[j, o:o + RG, :]
                    parts.append(acc)
                tok = parts[-1]
        s = jnp.concatenate(parts, axis=0).astype(BF16)
        return s, (_ortree(pltpu.bitcast(s, U32)) if 's1' in PINS else None)

    def stage_s3(r0, lg):
        tok = None
        res = []
        for gi, r in enumerate(range(r0, r0 + SB, RG)):
            s = [lg[(gi * W + w) * RG:(gi * W + w + 1) * RG] for w in range(W)]
            if r < HALO:
                row = r + lax.broadcasted_iota(I32, (RG, 128), 0)
                s = [s[0]] + [jnp.where(row >= DIL * w, s[w], -1e30) for w in range(1, W)]
            m = s[0]
            if GCH and res:
                m = fdep(m, res[-1][:, (NT - 1) * 128:])
            for w in range(1, W):
                m = jnp.maximum(m, s[w])
            e = [jnp.exp2((s[w] - m) * EXP2_SCALE) for w in range(W)]
            l = e[0]
            for w in range(1, W):
                l = l + e[w]
            if RCP:
                inv = pl.reciprocal(l, approx=True)
                inv = inv * (2.0 - l * inv)
            else:
                inv = 1.0 / l
            outs = []
            for j in range(NT):
                acc = e[0] * vb[j, HALO + r:HALO + r + RG, :]
                for w in range(1, W):
                    o = HALO - DIL * w + r
                    acc = acc + e[w] * vb[j, o:o + RG, :]
                outs.append(acc * inv)
            res.append(jnp.concatenate(outs, axis=1))
        o = pltpu.bitcast(jnp.concatenate(res, axis=0).astype(BF16), U32)
        obuf[r0 // 2:(r0 + SB) // 2, :] = o
        return _ortree(o) if 's3' in PINS else None

    def stage_o(n, h, toks):
        lhs = pltpu.bitcast(pin(wot[h * (D // 4):(h + 1) * (D // 4), :], toks), BF16)
        o = pltpu.bitcast(obuf[n * 64:(n + 1) * 64, :], BF16)
        return lax.dot_general(lhs, o, (((1,), (1,)), ((), ())), preferred_element_type=F32)

    def stage_e(n, out_t):
        c, hh = divmod(n, TM // 128)
        cols = slice(hh * 128, (hh + 1) * 128)
        if 'E' in SKIP:
            xt[c, :, cols] = out_t
            return None
        x = xt[c, :, cols] + out_t
        xt[c, :, cols] = x
        xc, v = _ln_stats(x)
        r1 = lax.rsqrt(v + EPS)
        r2 = lax.rsqrt(v * r1 * r1 + EPS)
        hv = (xc * (r1 * r2)).astype(BF16)
        ht[c, :, cols] = hv
        return _ortree(pltpu.bitcast(hv, U32)) if 'e' in PINS else None

    def phase_a(first):
        rsum = make_rsum()
        nslot = NRUN * (TM // RB)
        SPC = TM // RB
        NSUB = RB // SB
        if first:
            cp_x[0].wait()
            load_x(0)
            for h in range(2):
                stage_p(0, h)
            for i in range(NQP):
                cp_wq[i].wait()
                prep_w(0, 2 * i, 2 * i + 2)
            cp_x[1].wait()
            for cp in (cp_x[2], cp_w[2]):
                cp.start()
            stage_q(0, 0, 8, [])
            load_x(1)
            for h in range(2):
                stage_p(1, h)
            cp_w[1].wait()
            cp_x[2].wait()
            for cp in (cp_w[3], *cp_x[3:]):
                cp.start()
            stage_q(1, 0, 8, [])
            prep_w(1)
            load_x(2)
            for h in range(2):
                stage_p(2, h)
            cp_w[2].wait()
            cp_w1.start()
            stage_q(0, 8, 16, [])
            stage_q(2, 0, 8, [])
            prep_w(2)
            cp_w[3].wait()
            for c in range(3, NCH):
                cp_x[c].wait()
            cp_w2.start()
            stage_q(0, 16, 24, [])
            prep_wo()
            load_x(3)
        else:
            for h in range(2):
                stage_p(0, h)
            for h in range(2):
                stage_p(1, h)
            stage_q(0, 0, 24, [])
        lg_prev = None
        ohalf = {}
        ptok = {}
        carry = []
        for s in range(nslot + 4):
            c, i = divmod(s, SPC)
            do_q = (c + 1 < NRUN) and s < nslot
            s3_toks = []
            if lg_prev is not None and 'ATT' not in SKIP:
                for u in range(NSUB):
                    s3_toks.append(stage_s3((s - 1) * RB + u * SB, lg_prev[u * SB * W:(u + 1) * SB * W]))
            lg_prev = None
            e_tok = None
            if s >= 5 and (s - 5) % 2 == 0 and (s - 5) // 2 < nslot // 2:
                n = (s - 5) // 2
                e_tok = stage_e(n, jnp.concatenate([ohalf.pop((n, 0)), ohalf.pop((n, 1))], axis=0))
            p_tok = None
            if first and i == 0 and c >= 1 and c + 3 < NRUN:
                load_x(c + 3)
            if c + 2 < NRUN and i % 2 == 1 and s < nslot and not (first and c == 0):
                p_tok = stage_p(c + 2, i // 2)
            s1 = []
            if s < nslot and 'ATT' not in SKIP:
                s1 = [stage_s1(s * RB + u * SB) for u in range(NSUB)]
            half = max(1, NSUB // 2)
            pins1 = carry
            pins2 = s3_toks[:half]
            pinso = s3_toks[half:]
            pins3 = [e_tok] + [t for _, t in s1[:half]]
            carry = [p_tok]
            if first and c + 1 <= 2:
                t0, qs = 8 + 4 * i, [2, 2]
            else:
                t0, qs = 6 * i, [4, 2]
            opos = 1
            tt = t0
            for qi, qn in enumerate(qs + [0]):
                if qi == opos and s >= 3 and (s - 3) // 2 < nslot // 2:
                    n, h = divmod(s - 3, 2)
                    ohalf[(n, h)] = stage_o(n, h, [])
                if do_q and qn:
                    stage_q(c + 1, tt, tt + qn, [])
                tt += qn
            if s1:
                sc = jnp.concatenate([x for x, _ in s1], axis=0)
                lg_prev = jnp.dot(sc, rsum, preferred_element_type=F32)

    def phase_b(l):
        b1 = b1_ref[...].astype(F32)
        b2 = b2_ref[...].astype(F32)
        def body(m, carry):
            with jax.named_scope("b_iter"):
                rows = pl.ds(pl.multiple_of(m * TB, TB), TB)
                lhs = jnp.concatenate([ht[c, rows, :] for c in range(NCH)], axis=1)
                u = jnp.dot(lhs, w1[...], preferred_element_type=F32) + b1
                u = 0.5 * u * (1.0 + jnp.tanh(GELU_C * (u + 0.044715 * (u * u * u))))
                y = jnp.dot(u.astype(BF16), w2[...], preferred_element_type=F32) + b2
                for c in range(NCH):
                    xnew = xt[c, rows, :] + y[:, c * TM:(c + 1) * TM]
                    if l == 0:
                        xt[c, rows, :] = xnew
                    else:
                        stage[m, c * TM:(c + 1) * TM, :] = xnew.astype(BF16).T

                if l == 1:
                    pltpu.make_async_copy(stage.at[m], out_hbm.at[:, pl.ds(pl.multiple_of(m * TB, TB), TB)],
                                          sem_out.at[m]).start()
            return carry
        lax.fori_loop(0, NB, body, 0)

    def out_copy(m):
        return pltpu.make_async_copy(stage.at[m], out_hbm.at[:, pl.ds(m * TB, TB)], sem_out.at[m])

    for l in range(2):
        with jax.named_scope("phase_a"):
            phase_a(l == 0)
        if l == 0:
            cp_w1.wait()
            cp_w2.wait()
        if not ONLY_A:
            with jax.named_scope("phase_b"):
                phase_b(l)
    if ONLY_A:
        for m in range(NB):
            stage[m] = jnp.zeros((S, TB), BF16)
        stage[0, 0:TM, :] = ht[0, 0:TB, :]
    if ONLY_A:
        for m in range(NB):
            out_copy(m).start()
    for m in range(NB):
        out_copy(m).wait()


@jax.jit
def pallas_interleave_layers__sliding_local_dilated__mixer_token_mlp__prompt_kernel(
    A_x, A_wqkv, A_wo, B_x, B_w1, B_b1, B_w2, B_b2):
    del B_x
    x = A_x.reshape(S, D)
    any_spec = pl.BlockSpec(memory_space=pl.ANY)
    vmem_spec = pl.BlockSpec(memory_space=pltpu.VMEM)
    smem_spec = pl.BlockSpec(memory_space=pltpu.SMEM)
    scratch = [
        pltpu.VMEM((NCH, D, TM), F32),
        pltpu.VMEM((NCH, D, TM), BF16),
        pltpu.VMEM((4, D, D), BF16),
        pltpu.VMEM((D // 2, 3 * D), U32),
        pltpu.VMEM((D // 2, D), U32),
        pltpu.VMEM((S, F), BF16),
        pltpu.VMEM((F, S), BF16),
        pltpu.VMEM((NCH, TM, D), BF16),
        pltpu.VMEM((NCH, TM // 2, D), U32),
        pltpu.VMEM((NT, S, 128), F32),
        pltpu.VMEM((NT, S + HALO, 128), F32),
        pltpu.VMEM((NT, S + HALO, 128), F32),
        pltpu.VMEM((S // 2, D), U32),
        pltpu.VMEM((NB, S, TB), BF16),
        pltpu.SemaphoreType.DMA((NCH + 10,)),
        pltpu.SemaphoreType.DMA((NB,)),
    ]
    out = pl.pallas_call(
        _kernel,
        out_shape=jax.ShapeDtypeStruct((S, D), BF16),
        in_specs=[smem_spec, any_spec, any_spec, any_spec, any_spec, vmem_spec, any_spec, vmem_spec],
        out_specs=any_spec,
        scratch_shapes=scratch,
        compiler_params=pltpu.CompilerParams(vmem_limit_bytes=124 * 1024 * 1024),
    )(jnp.zeros((1,), jnp.int32), x, A_wqkv, A_wo, B_w1, B_b1.reshape(1, F), B_w2, B_b2.reshape(1, S))
    return out.reshape(1, S, D)
```

```python
import math

import jax
import jax.numpy as jnp
from jax import lax
import jax.experimental.pallas as pl
import jax.experimental.pallas.tpu as pltpu

S = 2048
D = 1024
F = 3584
H = 32
DH = D // H
W = 8
DIL = 2
HALO = 16
EPS = 1e-5
TM = 256
NCH = S // TM
TB = 128
NB = D // TB
NT = D // 128
RG = 8
RB = 64
NSLOT = S // RB
SPC = TM // RB
LAG = 2
OLAG = 3 + LAG
NQP = 4
NWP = 8
RW = D // NWP
NOP = NCH // 2
BF16 = jnp.bfloat16
F32 = jnp.float32
U32 = jnp.uint32
I32 = jnp.int32
EXP2_SCALE = (DH ** -0.5) * math.log2(math.e)
GELU_C = math.sqrt(2.0 / math.pi)


def _permute_cols(w):
    u = pltpu.bitcast(w, U32)
    tiles = [u[:, j * 128:(j + 1) * 128] for j in range(NT)]
    lane = lax.broadcasted_iota(I32, tiles[0].shape, 1)
    for tb, lb in ((2, 4), (1, 3), (0, 2)):
        keep = ((lane >> lb) & 1) == 0
        new = list(tiles)
        for j in range(NT):
            if (j >> tb) & 1:
                continue
            a, b = tiles[j], tiles[j | (1 << tb)]
            new[j] = jnp.where(keep, a, pltpu.roll(b, 1 << lb, 1))
            new[j | (1 << tb)] = jnp.where(keep, pltpu.roll(a, 128 - (1 << lb), 1), b)
        tiles = new
    return jnp.concatenate(tiles, axis=1)


def _col_stats(load):
    acc = None
    for r in range(0, D, 256):
        p = jnp.sum(load(r, r + 256).reshape(32, 8, 128), axis=0)
        acc = p if acc is None else acc + p
    m = jnp.sum(acc, axis=0, keepdims=True) * (1.0 / D)
    acc = None
    for r in range(0, D, 128):
        xc = load(r, r + 128) - m
        p = jnp.sum((xc * xc).reshape(16, 8, 128), axis=0)
        acc = p if acc is None else acc + p
    v = jnp.sum(acc, axis=0, keepdims=True) * (1.0 / D)
    return m, v


def _kernel(x_hbm, wqkv_hbm, wo_hbm, w1_hbm, b1_hbm, w2_hbm, b2_hbm, out_hbm,
            b1_raw, b2_raw, b1_ref, b2_ref, xt, ht, wraw, wqkv, wot, w1, w2, xin, xn,
            qb, kb, vb, obuf, stage, sem_in, sem_out):
    cp_x = [pltpu.make_async_copy(x_hbm.at[pl.ds(c * TM, TM), :], xin.at[c], sem_in.at[c])
            for c in range(NCH)]
    qp = D // NQP
    cp_wq = [pltpu.make_async_copy(wqkv_hbm.at[pl.ds(i * qp, qp), pl.ds(0, D)],
                                   wraw.at[0, pl.ds(i * qp, qp), :], sem_in.at[NCH + i])
             for i in range(NQP)]
    sb = NCH + NQP
    cp_wk = pltpu.make_async_copy(wqkv_hbm.at[:, pl.ds(D, D)], wraw.at[1], sem_in.at[sb])
    cp_wv = pltpu.make_async_copy(wqkv_hbm.at[:, pl.ds(2 * D, D)], wraw.at[2], sem_in.at[sb + 1])
    cp_wo = pltpu.make_async_copy(wo_hbm, wraw.at[3], sem_in.at[sb + 2])
    cp_w1 = pltpu.make_async_copy(w1_hbm, w1, sem_in.at[sb + 3])
    cp_w2 = pltpu.make_async_copy(w2_hbm, w2, sem_in.at[sb + 4])
    cp_b1 = pltpu.make_async_copy(b1_hbm, b1_raw, sem_in.at[sb + 5])
    cp_b2 = pltpu.make_async_copy(b2_hbm, b2_raw, sem_in.at[sb + 6])
    for cp in (cp_x[0], *cp_wq, cp_x[1], cp_x[2], cp_wk):
        cp.start()
    for b in (kb, vb):
        b[:, 0:HALO, :] = jnp.zeros((NT, HALO, 128), F32)

    def prep_w(t, i0=0, i1=NWP):
        for i in range(i0, i1):
            wqkv[i * RW // 2:(i + 1) * RW // 2, t * D:(t + 1) * D] = _permute_cols(wraw[t, i * RW:(i + 1) * RW, :])

    def prep_wo():
        wo_t = wraw[3].T
        for i in range(NWP):
            wot[i * RW // 2:(i + 1) * RW // 2, :] = _permute_cols(wo_t[i * RW:(i + 1) * RW, :])

    def load_x(c):
        xt[c] = xin[c].astype(F32).T

    def stage_p(c, h):
        cols = slice(h * 128, (h + 1) * 128)
        load = lambda r0, r1: xt[c, r0:r1, cols]
        m, v = _col_stats(load)
        r = lax.rsqrt(v + EPS)
        mr = m * r
        for j in range(NT):
            y = (load(j * 128, (j + 1) * 128) * r - mr).astype(BF16)
            xn[c, h * 64:(h + 1) * 64, j * 128:(j + 1) * 128] = pltpu.bitcast(y.T, U32)

    def store_qkv(c, t, piece):
        kind, j = divmod(t, NT)
        if kind == 0:
            qb[j, c * TM:(c + 1) * TM, :] = piece
        else:
            (kb if kind == 1 else vb)[j, HALO + c * TM:HALO + (c + 1) * TM, :] = piece

    def stage_q(c, t0, t1):
        res = jnp.dot(pltpu.bitcast(xn[c], BF16), pltpu.bitcast(wqkv[:, t0 * 128:t1 * 128], BF16),
                      preferred_element_type=F32)
        for t in range(t0, t1):
            store_qkv(c, t, res[:, (t - t0) * 128:(t - t0 + 1) * 128])

    def stage_s1(r0):
        parts = []
        for r in range(r0, r0 + RB, RG):
            q = [qb[j, r:r + RG, :] for j in range(NT)]
            for w in range(W):
                o = HALO - DIL * w + r
                acc = q[0] * kb[0, o:o + RG, :]
                for j in range(1, NT):
                    acc = acc + q[j] * kb[j, o:o + RG, :]
                parts.append(acc)
        return jnp.concatenate(parts, axis=0).astype(BF16)

    def stage_s3(r0, lg):
        res = []
        for gi, r in enumerate(range(r0, r0 + RB, RG)):
            s = [lg[(gi * W + w) * RG:(gi * W + w + 1) * RG] for w in range(W)]
            if r < HALO:
                row = r + lax.broadcasted_iota(I32, (RG, 128), 0)
                s = [s[0]] + [jnp.where(row >= DIL * w, s[w], -1e30) for w in range(1, W)]
            m = s[0]
            for w in range(1, W):
                m = jnp.maximum(m, s[w])
            e = [jnp.exp2((s[w] - m) * EXP2_SCALE) for w in range(W)]
            l = e[0]
            for w in range(1, W):
                l = l + e[w]
            inv = pl.reciprocal(l, approx=True)
            inv = inv * (2.0 - l * inv)
            outs = []
            for j in range(NT):
                acc = e[0] * vb[j, HALO + r:HALO + r + RG, :]
                for w in range(1, W):
                    o = HALO - DIL * w + r
                    acc = acc + e[w] * vb[j, o:o + RG, :]
                outs.append(acc * inv)
            res.append(jnp.concatenate(outs, axis=1))
        obuf[r0 // 2:(r0 + RB) // 2, :] = pltpu.bitcast(jnp.concatenate(res, axis=0).astype(BF16), U32)

    def stage_o(n, h):
        lhs = pltpu.bitcast(wot[h * (D // 4):(h + 1) * (D // 4), :], BF16)
        o = pltpu.bitcast(obuf[n * 64:(n + 1) * 64, :], BF16)
        return lax.dot_general(lhs, o, (((1,), (1,)), ((), ())), preferred_element_type=F32)

    def stage_e(n, out_t):
        c, hh = divmod(n, TM // 128)
        cols = slice(hh * 128, (hh + 1) * 128)
        xt[c, :, cols] = xt[c, :, cols] + out_t
        load = lambda r0, r1: xt[c, r0:r1, cols]
        m, v = _col_stats(load)
        r1 = lax.rsqrt(v + EPS)
        r = r1 * lax.rsqrt(v * r1 * r1 + EPS)
        mr = m * r
        for j in range(0, D, 64):
            ht[c, j // 2:(j + 64) // 2, cols] = pltpu.bitcast((load(j, j + 64) * r - mr).astype(BF16), U32)

    def phase_a(first):
        li = lax.broadcasted_iota(I32, (128, 128), 0) >> 2
        lj = lax.broadcasted_iota(I32, (128, 128), 1) >> 2
        rsum = (li == lj).astype(BF16)
        if first:
            cp_x[0].wait()
            load_x(0)
            for h in range(2):
                stage_p(0, h)
            acc = None
            for i in range(NQP):
                cp_wq[i].wait()
                if i == NQP - 1:
                    cp_x[1].wait()
                prep_w(0, 2 * i, 2 * i + 2)
                part = jnp.dot(pltpu.bitcast(xn[0, :, i * qp:(i + 1) * qp], BF16),
                               pltpu.bitcast(wqkv[i * qp // 2:(i + 1) * qp // 2, 0:D], BF16),
                               preferred_element_type=F32)
                acc = part if acc is None else acc + part
            load_x(1)
            for h in range(2):
                stage_p(1, h)
            for j in range(NT):
                store_qkv(0, j, acc[:, j * 128:(j + 1) * 128])
            cp_x[2].wait()
            cp_wv.start()
            stage_q(1, 0, NT)
            load_x(2)
            for h in range(2):
                stage_p(2, h)
            cp_wk.wait()
            for cp in (cp_wo, *cp_x[3:]):
                cp.start()
            stage_q(2, 0, NT)
            prep_w(1)
            cp_wv.wait()
            for cp in (cp_w1, cp_b1, cp_b2):
                cp.start()
            stage_q(0, NT, 2 * NT)
            prep_w(2)
            cp_wo.wait()
            for c in range(3, NCH):
                cp_x[c].wait()
            cp_w2.start()
            stage_q(0, 2 * NT, 3 * NT)
            prep_wo()
            load_x(3)
        else:
            for c in range(2):
                for h in range(2):
                    stage_p(c, h)
            stage_q(0, 0, 3 * NT)

        partial, logits, ohalf = {}, {}, {}
        for s in range(NSLOT + OLAG + 3):
            c, i = divmod(s, SPC)
            b3 = s - 1 - LAG
            if 0 <= b3 < NSLOT:
                stage_s3(b3 * RB, logits.pop(b3))
            if s >= OLAG + 2 and (s - OLAG) % 2 == 0 and (s - OLAG - 2) // 2 < S // 128:
                n = (s - OLAG - 2) // 2
                stage_e(n, jnp.concatenate([ohalf.pop((n, 0)), ohalf.pop((n, 1))], axis=0))
            if first and i == 0 and c >= 1 and c + 3 < NCH:
                load_x(c + 3)
            if c + 2 < NCH and i % 2 == 0 and not (first and c == 0):
                stage_p(c + 2, i // 2)
            if s < NSLOT:
                partial[s] = stage_s1(s * RB)
            if first and c + 1 <= 2:
                t0, n0, n1 = NT + 4 * i, 2, 2
            else:
                t0, n0, n1 = 6 * i, 4, 2
            do_q = c + 1 < NCH
            if do_q:
                stage_q(c + 1, t0, t0 + n0)
            if s >= OLAG and (s - OLAG) // 2 < S // 128:
                n, h = divmod(s - OLAG, 2)
                ohalf[(n, h)] = stage_o(n, h)
            if do_q:
                stage_q(c + 1, t0 + n0, t0 + n0 + n1)
            br = s - LAG
            if 0 <= br < NSLOT:
                logits[br] = jnp.dot(partial.pop(br), rsum, preferred_element_type=F32)

    def phase_b(last):
        b1 = b1_ref[...]
        b2 = b2_ref[...]

        def body(m, carry):
            rows = pl.ds(pl.multiple_of(m * TB, TB), TB)
            prow = pl.ds(pl.multiple_of(m * (TB // 2), TB // 2), TB // 2)
            lhs = pltpu.bitcast(jnp.concatenate([ht[c, prow, :] for c in range(NCH)], axis=1), BF16)
            u = jnp.dot(lhs, w1[...], preferred_element_type=F32) + b1
            u = 0.5 * u * (1.0 + jnp.tanh(GELU_C * (u + 0.044715 * (u * u * u))))
            y = jnp.dot(u.astype(BF16), w2[...], preferred_element_type=F32) + b2
            for c in range(NCH):
                xnew = xt[c, rows, :] + y[:, c * TM:(c + 1) * TM]
                if not last:
                    xt[c, rows, :] = xnew
                else:
                    stage[m, c * TM:(c + 1) * TM, :] = xnew.astype(BF16).T
                    if c % 2 == 1:
                        pltpu.make_async_copy(
                            stage.at[m, pl.ds((c - 1) * TM, 2 * TM), :],
                            out_hbm.at[pl.ds((c - 1) * TM, 2 * TM), rows],
                            sem_out.at[m * NOP + c // 2]).start()
            return carry
        lax.fori_loop(0, NB, body, 0)

    phase_a(True)
    cp_w1.wait()
    cp_w2.wait()
    cp_b1.wait()
    cp_b2.wait()
    b1_ref[...] = b1_raw[...].astype(F32).reshape(1, F)
    b2_ref[...] = b2_raw[...].astype(F32).reshape(1, S)
    phase_b(False)
    phase_a(False)
    phase_b(True)
    for m in range(NB):
        for k in range(NOP):
            pltpu.make_async_copy(stage.at[m, pl.ds(k * 2 * TM, 2 * TM), :],
                                  out_hbm.at[pl.ds(k * 2 * TM, 2 * TM), pl.ds(m * TB, TB)],
                                  sem_out.at[m * NOP + k]).wait()


@jax.jit
def pallas_interleave_layers__sliding_local_dilated__mixer_token_mlp__prompt_kernel(
    A_x: jax.Array,
    A_wqkv: jax.Array,
    A_wo: jax.Array,
    B_x: jax.Array,
    B_w1: jax.Array,
    B_b1: jax.Array,
    B_w2: jax.Array,
    B_b2: jax.Array,
):
    del B_x
    scratch = [
        pltpu.VMEM((F,), BF16),
        pltpu.VMEM((S,), BF16),
        pltpu.VMEM((1, F), F32),
        pltpu.VMEM((1, S), F32),
        pltpu.VMEM((NCH, D, TM), F32),
        pltpu.VMEM((NCH, D // 2, TM), U32),
        pltpu.VMEM((4, D, D), BF16),
        pltpu.VMEM((D // 2, 3 * D), U32),
        pltpu.VMEM((D // 2, D), U32),
        pltpu.VMEM((S, F), BF16),
        pltpu.VMEM((F, S), BF16),
        pltpu.VMEM((NCH, TM, D), BF16),
        pltpu.VMEM((NCH, TM // 2, D), U32),
        pltpu.VMEM((NT, S, 128), F32),
        pltpu.VMEM((NT, HALO + S, 128), F32),
        pltpu.VMEM((NT, HALO + S, 128), F32),
        pltpu.VMEM((S // 2, D), U32),
        pltpu.VMEM((NB, S, TB), BF16),
        pltpu.SemaphoreType.DMA((NCH + NQP + 7,)),
        pltpu.SemaphoreType.DMA((NB * NOP,)),
    ]
    out = pl.pallas_call(
        _kernel,
        out_shape=jax.ShapeDtypeStruct((S, D), BF16),
        in_specs=[pl.BlockSpec(memory_space=pl.ANY)] * 7,
        out_specs=pl.BlockSpec(memory_space=pl.ANY),
        scratch_shapes=scratch,
        compiler_params=pltpu.CompilerParams(vmem_limit_bytes=124 * 1024 * 1024),
    )(A_x.reshape(S, D), A_wqkv, A_wo, B_w1, B_b1, B_w2, B_b2)
    return out.reshape(1, S, D)
```

```python
import math

import jax
import jax.numpy as jnp
from jax import lax
import jax.experimental.pallas as pl
import jax.experimental.pallas.tpu as pltpu

S = 2048
D = 1024
F = 3584
H = 32
DH = D // H
W = 8
DIL = 2
HALO = 16
EPS = 1e-5
TM = 256
NCH = S // TM
TB = 128
NB = D // TB
NT = D // 128
RG = 8
RB = 64
NSLOT = S // RB
SPC = TM // RB
LAG = 2
OLAG = 3 + LAG
NQP = 4
NWP = 8
RW = D // NWP
NOP = NCH // 2
BF16 = jnp.bfloat16
F32 = jnp.float32
U32 = jnp.uint32
I32 = jnp.int32
EXP2_SCALE = (DH ** -0.5) * math.log2(math.e)
GELU_C = math.sqrt(2.0 / math.pi)


def _permute_cols(w):
    u = pltpu.bitcast(w, U32)
    tiles = [u[:, j * 128:(j + 1) * 128] for j in range(NT)]
    lane = lax.broadcasted_iota(I32, tiles[0].shape, 1)
    for tb, lb in ((2, 4), (1, 3), (0, 2)):
        keep = ((lane >> lb) & 1) == 0
        new = list(tiles)
        for j in range(NT):
            if (j >> tb) & 1:
                continue
            a, b = tiles[j], tiles[j | (1 << tb)]
            new[j] = jnp.where(keep, a, pltpu.roll(b, 1 << lb, 1))
            new[j | (1 << tb)] = jnp.where(keep, pltpu.roll(a, 128 - (1 << lb), 1), b)
        tiles = new
    return jnp.concatenate(tiles, axis=1)


def _col_stats(load):
    acc = None
    for r in range(0, D, 256):
        p = jnp.sum(load(r, r + 256).reshape(32, 8, 128), axis=0)
        acc = p if acc is None else acc + p
    m = jnp.sum(acc, axis=0, keepdims=True) * (1.0 / D)
    acc = None
    for r in range(0, D, 128):
        xc = load(r, r + 128) - m
        p = jnp.sum((xc * xc).reshape(16, 8, 128), axis=0)
        acc = p if acc is None else acc + p
    v = jnp.sum(acc, axis=0, keepdims=True) * (1.0 / D)
    return m, v


def _kernel(x_hbm, wqkv_hbm, wo_hbm, w1_hbm, b1_hbm, w2_hbm, b2_hbm, out_hbm,
            b1_raw, b2_raw, b1_ref, b2_ref, xt, mp, se, pacc, wraw, wqkv, wot, w1, w2, xin, xn,
            qb, kb, vb, obuf, stage, sem_in, sem_out):
    cp_x = [pltpu.make_async_copy(x_hbm.at[pl.ds(c * TM, TM), :], xin.at[c], sem_in.at[c])
            for c in range(NCH)]
    qp = D // NQP
    cp_wq = [pltpu.make_async_copy(wqkv_hbm.at[pl.ds(i * qp, qp), pl.ds(0, D)],
                                   wraw.at[0, pl.ds(i * qp, qp), :], sem_in.at[NCH + i])
             for i in range(NQP)]
    sb = NCH + NQP
    cp_wk = pltpu.make_async_copy(wqkv_hbm.at[:, pl.ds(D, D)], wraw.at[1], sem_in.at[sb])
    cp_wv = pltpu.make_async_copy(wqkv_hbm.at[:, pl.ds(2 * D, D)], wraw.at[2], sem_in.at[sb + 1])
    cp_wo = pltpu.make_async_copy(wo_hbm, wraw.at[3], sem_in.at[sb + 2])
    cp_w1 = pltpu.make_async_copy(w1_hbm, w1, sem_in.at[sb + 3])
    cp_w2 = pltpu.make_async_copy(w2_hbm, w2, sem_in.at[sb + 4])
    cp_b1 = pltpu.make_async_copy(b1_hbm, b1_raw, sem_in.at[sb + 5])
    cp_b2 = pltpu.make_async_copy(b2_hbm, b2_raw, sem_in.at[sb + 6])
    for cp in (cp_x[0], *cp_wq, cp_x[1], cp_x[2], cp_wk):
        cp.start()
    for b in (kb, vb):
        b[:, 0:HALO, :] = jnp.zeros((NT, HALO, 128), F32)

    def prep_w(t, i0=0, i1=NWP):
        for i in range(i0, i1):
            wqkv[i * RW // 2:(i + 1) * RW // 2, t * D:(t + 1) * D] = _permute_cols(wraw[t, i * RW:(i + 1) * RW, :])

    def prep_wo():
        wo_t = wraw[3].T
        for i in range(NWP):
            wot[i * RW // 2:(i + 1) * RW // 2, :] = _permute_cols(wo_t[i * RW:(i + 1) * RW, :])

    def load_x(c):
        xt[c] = xin[c].astype(F32).T

    def colsum(p):
        return jnp.sum(p, axis=0, keepdims=True) * (1.0 / D)

    def stage_p(c, h, first):
        cols = slice(h * 128, (h + 1) * 128)
        load = lambda r0, r1: xt[c, r0:r1, cols]
        if first:
            m, v = _col_stats(load)
        else:
            dm = colsum(pacc[0, c, :, cols])
            m = se[2, c, 0:1, cols] + dm
            v = jnp.maximum(colsum(pacc[1, c, :, cols]) - dm * dm, 0.0)
        mp[2 * c + h] = jnp.broadcast_to(m, (8, 128))
        r = lax.rsqrt(v + EPS)
        mr = m * r
        for j in range(NT):
            y = (load(j * 128, (j + 1) * 128) * r - mr).astype(BF16)
            xn[c, h * 64:(h + 1) * 64, j * 128:(j + 1) * 128] = pltpu.bitcast(y.T, U32)

    def store_qkv(c, t, piece):
        kind, j = divmod(t, NT)
        if kind == 0:
            qb[j, c * TM:(c + 1) * TM, :] = piece
        else:
            (kb if kind == 1 else vb)[j, HALO + c * TM:HALO + (c + 1) * TM, :] = piece

    def stage_q(c, t0, t1):
        res = jnp.dot(pltpu.bitcast(xn[c], BF16), pltpu.bitcast(wqkv[:, t0 * 128:t1 * 128], BF16),
                      preferred_element_type=F32)
        for t in range(t0, t1):
            store_qkv(c, t, res[:, (t - t0) * 128:(t - t0 + 1) * 128])

    def stage_s1(r0):
        parts = []
        for r in range(r0, r0 + RB, RG):
            q = [qb[j, r:r + RG, :] for j in range(NT)]
            for w in range(W):
                o = HALO - DIL * w + r
                acc = q[0] * kb[0, o:o + RG, :]
                for j in range(1, NT):
                    acc = acc + q[j] * kb[j, o:o + RG, :]
                parts.append(acc)
        return jnp.concatenate(parts, axis=0).astype(BF16)

    def stage_s3(r0, lg):
        res = []
        for gi, r in enumerate(range(r0, r0 + RB, RG)):
            s = [lg[(gi * W + w) * RG:(gi * W + w + 1) * RG] for w in range(W)]
            if r < HALO:
                row = r + lax.broadcasted_iota(I32, (RG, 128), 0)
                s = [s[0]] + [jnp.where(row >= DIL * w, s[w], -1e30) for w in range(1, W)]
            m = s[0]
            for w in range(1, W):
                m = jnp.maximum(m, s[w])
            e = [jnp.exp2((s[w] - m) * EXP2_SCALE) for w in range(W)]
            l = e[0]
            for w in range(1, W):
                l = l + e[w]
            inv = pl.reciprocal(l, approx=True)
            inv = inv * (2.0 - l * inv)
            outs = []
            for j in range(NT):
                acc = e[0] * vb[j, HALO + r:HALO + r + RG, :]
                for w in range(1, W):
                    o = HALO - DIL * w + r
                    acc = acc + e[w] * vb[j, o:o + RG, :]
                outs.append(acc * inv)
            res.append(jnp.concatenate(outs, axis=1))
        obuf[r0 // 2:(r0 + RB) // 2, :] = pltpu.bitcast(jnp.concatenate(res, axis=0).astype(BF16), U32)

    def stage_o(n, h):
        lhs = pltpu.bitcast(wot[h * (D // 4):(h + 1) * (D // 4), :], BF16)
        o = pltpu.bitcast(obuf[n * 64:(n + 1) * 64, :], BF16)
        return lax.dot_general(lhs, o, (((1,), (1,)), ((), ())), preferred_element_type=F32)

    def stage_res(n, h, res):
        c, hh = divmod(n, TM // 128)
        rows = slice(h * (D // 2), (h + 1) * (D // 2))
        cols = slice(hh * 128, (hh + 1) * 128)
        xnew = xt[c, rows, cols] + res
        xt[c, rows, cols] = xnew
        d = xnew.reshape(D // 16, 8, 128) - mp[n]
        return jnp.sum(d, axis=0), jnp.sum(d * d, axis=0)

    def stage_e(n, s1, s2):
        c, hh = divmod(n, TM // 128)
        cols = slice(hh * 128, (hh + 1) * 128)
        dm = colsum(s1)
        m = mp[n, 0:1, :] + dm
        v = jnp.maximum(colsum(s2) - dm * dm, 0.0)
        r1 = lax.rsqrt(v + EPS)
        r = r1 * lax.rsqrt(v * r1 * r1 + EPS)
        se[0, c, :, cols] = jnp.broadcast_to(r, (8, 128))
        se[1, c, :, cols] = jnp.broadcast_to(m * r, (8, 128))
        se[2, c, :, cols] = jnp.broadcast_to(m, (8, 128))

    def phase_a(first):
        li = lax.broadcasted_iota(I32, (128, 128), 0) >> 2
        lj = lax.broadcasted_iota(I32, (128, 128), 1) >> 2
        rsum = (li == lj).astype(BF16)
        if first:
            cp_x[0].wait()
            load_x(0)
            for h in range(2):
                stage_p(0, h, True)
            acc = None
            for i in range(NQP):
                cp_wq[i].wait()
                if i == NQP - 1:
                    cp_x[1].wait()
                prep_w(0, 2 * i, 2 * i + 2)
                part = jnp.dot(pltpu.bitcast(xn[0, :, i * qp:(i + 1) * qp], BF16),
                               pltpu.bitcast(wqkv[i * qp // 2:(i + 1) * qp // 2, 0:D], BF16),
                               preferred_element_type=F32)
                acc = part if acc is None else acc + part
            load_x(1)
            for h in range(2):
                stage_p(1, h, True)
            for j in range(NT):
                store_qkv(0, j, acc[:, j * 128:(j + 1) * 128])
            cp_x[2].wait()
            cp_wv.start()
            stage_q(1, 0, NT)
            load_x(2)
            for h in range(2):
                stage_p(2, h, True)
            cp_wk.wait()
            for cp in (cp_wo, *cp_x[3:]):
                cp.start()
            stage_q(2, 0, NT)
            prep_w(1)
            cp_wv.wait()
            for cp in (cp_w1, cp_b1, cp_b2):
                cp.start()
            stage_q(0, NT, 2 * NT)
            prep_w(2)
            cp_wo.wait()
            for c in range(3, NCH):
                cp_x[c].wait()
            cp_w2.start()
            stage_q(0, 2 * NT, 3 * NT)
            prep_wo()
            load_x(3)
        else:
            for c in range(2):
                for h in range(2):
                    stage_p(c, h, False)
            stage_q(0, 0, 3 * NT)

        seq = []
        nq_slots = (NCH - 1) * SPC
        for s in range(nq_slots):
            c, i = divmod(s, SPC)
            if first and c + 1 <= 2:
                t0, n0, n1 = NT + 4 * i, 2, 2
            else:
                t0, n0, n1 = 6 * i, 4, 2
            seq.append(('q', c + 1, t0, t0 + n0))
            if s >= OLAG:
                seq.append(('o',) + divmod(s - OLAG, 2))
            seq.append(('q', c + 1, t0 + n0, t0 + n0 + n1))
            if s >= LAG:
                seq.append(('r', s - LAG))
        r_next = nq_slots - LAG
        o_next = nq_slots - OLAG
        while o_next < S // 64:
            seq.append(('o',) + divmod(o_next, 2))
            o_next += 1
            if r_next < NSLOT:
                seq.append(('r', r_next))
                r_next += 1

        logits, sums = {}, {}
        done_p = {0, 1, 2} if first else {0, 1}
        done_x = {0, 1, 2, 3}
        done_s3 = set()
        for op in seq:
            if op[0] == 'q':
                _, c, t0, t1 = op
                for cc in (c, c + 1):
                    if cc < NCH and cc not in done_p:
                        if first and cc not in done_x:
                            load_x(cc)
                            done_x.add(cc)
                        for h in range(2):
                            stage_p(cc, h, first)
                        done_p.add(cc)
                stage_q(c, t0, t1)
            elif op[0] == 'r':
                b = op[1]
                logits[b] = jnp.dot(stage_s1(b * RB), rsum, preferred_element_type=F32)
            else:
                _, n, h = op
                for b in (2 * n, 2 * n + 1):
                    if b not in done_s3:
                        stage_s3(b * RB, logits.pop(b))
                        done_s3.add(b)
                sums[(n, h)] = stage_res(n, h, stage_o(n, h))
                if h == 1:
                    a, b = sums.pop((n, 0)), sums.pop((n, 1))
                    stage_e(n, a[0] + b[0], a[1] + b[1])

    def phase_b(last):
        b1 = b1_ref[...]
        b2 = b2_ref[...]

        if not last:
            pacc[...] = jnp.zeros(pacc.shape, F32)

        def body(m, carry):
            rows = pl.ds(pl.multiple_of(m * TB, TB), TB)
            lhs = jnp.concatenate(
                [(xt[c, rows, :].reshape(TB // 8, 8, TM) * se[0, c] - se[1, c]).reshape(TB, TM).astype(BF16)
                 for c in range(NCH)], axis=1)
            u = jnp.dot(lhs, w1[...], preferred_element_type=F32) + b1
            u = 0.5 * u * (1.0 + jnp.tanh(GELU_C * (u + 0.044715 * (u * u * u))))
            y = jnp.dot(u.astype(BF16), w2[...], preferred_element_type=F32) + b2
            for c in range(NCH):
                xnew = xt[c, rows, :] + y[:, c * TM:(c + 1) * TM]
                if not last:
                    xt[c, rows, :] = xnew
                    d = xnew.reshape(TB // 8, 8, TM) - se[2, c]
                    pacc[0, c] = pacc[0, c] + jnp.sum(d, axis=0)
                    pacc[1, c] = pacc[1, c] + jnp.sum(d * d, axis=0)
                else:
                    stage[m, c * TM:(c + 1) * TM, :] = xnew.astype(BF16).T
                    if c % 2 == 1:
                        pltpu.make_async_copy(
                            stage.at[m, pl.ds((c - 1) * TM, 2 * TM), :],
                            out_hbm.at[pl.ds((c - 1) * TM, 2 * TM), rows],
                            sem_out.at[m * NOP + c // 2]).start()
            return carry
        lax.fori_loop(0, NB, body, 0)

    phase_a(True)
    cp_w1.wait()
    cp_w2.wait()
    cp_b1.wait()
    cp_b2.wait()
    b1_ref[...] = b1_raw[...].astype(F32).reshape(1, F)
    b2_ref[...] = b2_raw[...].astype(F32).reshape(1, S)
    phase_b(False)
    phase_a(False)
    phase_b(True)
    for m in range(NB):
        for k in range(NOP):
            pltpu.make_async_copy(stage.at[m, pl.ds(k * 2 * TM, 2 * TM), :],
                                  out_hbm.at[pl.ds(k * 2 * TM, 2 * TM), pl.ds(m * TB, TB)],
                                  sem_out.at[m * NOP + k]).wait()


@jax.jit
def pallas_interleave_layers__sliding_local_dilated__mixer_token_mlp__prompt_kernel(
    A_x: jax.Array,
    A_wqkv: jax.Array,
    A_wo: jax.Array,
    B_x: jax.Array,
    B_w1: jax.Array,
    B_b1: jax.Array,
    B_w2: jax.Array,
    B_b2: jax.Array,
):
    del B_x
    scratch = [
        pltpu.VMEM((F,), BF16),
        pltpu.VMEM((S,), BF16),
        pltpu.VMEM((1, F), F32),
        pltpu.VMEM((1, S), F32),
        pltpu.VMEM((NCH, D, TM), F32),
        pltpu.VMEM((S // 128, 8, 128), F32),
        pltpu.VMEM((3, NCH, 8, TM), F32),
        pltpu.VMEM((2, NCH, 8, TM), F32),
        pltpu.VMEM((4, D, D), BF16),
        pltpu.VMEM((D // 2, 3 * D), U32),
        pltpu.VMEM((D // 2, D), U32),
        pltpu.VMEM((S, F), BF16),
        pltpu.VMEM((F, S), BF16),
        pltpu.VMEM((NCH, TM, D), BF16),
        pltpu.VMEM((NCH, TM // 2, D), U32),
        pltpu.VMEM((NT, S, 128), F32),
        pltpu.VMEM((NT, HALO + S, 128), F32),
        pltpu.VMEM((NT, HALO + S, 128), F32),
        pltpu.VMEM((S // 2, D), U32),
        pltpu.VMEM((NB, S, TB), BF16),
        pltpu.SemaphoreType.DMA((NCH + NQP + 7,)),
        pltpu.SemaphoreType.DMA((NB * NOP,)),
    ]
    out = pl.pallas_call(
        _kernel,
        out_shape=jax.ShapeDtypeStruct((S, D), BF16),
        in_specs=[pl.BlockSpec(memory_space=pl.ANY)] * 7,
        out_specs=pl.BlockSpec(memory_space=pl.ANY),
        scratch_shapes=scratch,
        compiler_params=pltpu.CompilerParams(vmem_limit_bytes=124 * 1024 * 1024),
    )(A_x.reshape(S, D), A_wqkv, A_wo, B_w1, B_b1, B_w2, B_b2)
    return out.reshape(1, S, D)
```

```python
import math

import jax
import jax.numpy as jnp
from jax import lax
import jax.experimental.pallas as pl
import jax.experimental.pallas.tpu as pltpu

S = 2048
D = 1024
F = 3584
H = 32
DH = D // H
W = 8
DIL = 2
HALO = 16
EPS = 1e-5
TM = 256
NCH = S // TM
TB = 128
NB = D // TB
NT = D // 128
RG = 8
RB = 64
NSLOT = S // RB
SPC = TM // RB
LAG = 2
OLAG = 3 + LAG
NQP = 4
NWP = 8
RW = D // NWP
NOP = NCH // 2
BF16 = jnp.bfloat16
F32 = jnp.float32
U32 = jnp.uint32
I32 = jnp.int32
EXP2_SCALE = (DH ** -0.5) * math.log2(math.e)
GELU_C = math.sqrt(2.0 / math.pi)


def _permute_cols(w):
    u = pltpu.bitcast(w, U32)
    tiles = [u[:, j * 128:(j + 1) * 128] for j in range(NT)]
    lane = lax.broadcasted_iota(I32, tiles[0].shape, 1)
    for tb, lb in ((2, 4), (1, 3), (0, 2)):
        keep = ((lane >> lb) & 1) == 0
        new = list(tiles)
        for j in range(NT):
            if (j >> tb) & 1:
                continue
            a, b = tiles[j], tiles[j | (1 << tb)]
            new[j] = jnp.where(keep, a, pltpu.roll(b, 1 << lb, 1))
            new[j | (1 << tb)] = jnp.where(keep, pltpu.roll(a, 128 - (1 << lb), 1), b)
        tiles = new
    return jnp.concatenate(tiles, axis=1)


def _kernel(x_hbm, wqkv_hbm, wo_hbm, w1_hbm, b1_hbm, w2_hbm, b2_hbm, out_hbm,
            b1_raw, b2_raw, b1_ref, b2_ref, xt, mp, se, pacc, wraw, wqkv, wot, w1, w2, xin, xn,
            qb, kb, vb, obuf, stage, sem_in, sem_out):
    cp_x = [pltpu.make_async_copy(x_hbm.at[pl.ds(c * TM, TM), :], xin.at[c], sem_in.at[c])
            for c in range(NCH)]
    qp = D // NQP
    cp_wq = [pltpu.make_async_copy(wqkv_hbm.at[pl.ds(i * qp, qp), pl.ds(0, D)],
                                   wraw.at[0, pl.ds(i * qp, qp), :], sem_in.at[NCH + i])
             for i in range(NQP)]
    sb = NCH + NQP
    cp_wk = pltpu.make_async_copy(wqkv_hbm.at[:, pl.ds(D, D)], wraw.at[1], sem_in.at[sb])
    cp_wv = pltpu.make_async_copy(wqkv_hbm.at[:, pl.ds(2 * D, D)], wraw.at[2], sem_in.at[sb + 1])
    cp_wo = pltpu.make_async_copy(wo_hbm, wraw.at[3], sem_in.at[sb + 2])
    cp_w1 = pltpu.make_async_copy(w1_hbm, w1, sem_in.at[sb + 3])
    cp_w2 = pltpu.make_async_copy(w2_hbm, w2, sem_in.at[sb + 4])
    cp_b1 = pltpu.make_async_copy(b1_hbm, b1_raw, sem_in.at[sb + 5])
    cp_b2 = pltpu.make_async_copy(b2_hbm, b2_raw, sem_in.at[sb + 6])
    for cp in (cp_x[0], *cp_wq, cp_x[1], cp_x[2], cp_wk, cp_wv, cp_wo, *cp_x[3:]):
        cp.start()
    for b in (kb, vb):
        b[:, 0:HALO, :] = jnp.zeros((NT, HALO, 128), F32)

    def prep_w(t, i0=0, i1=NWP):
        for i in range(i0, i1):
            wqkv[i * RW // 2:(i + 1) * RW // 2, t * D:(t + 1) * D] = _permute_cols(wraw[t, i * RW:(i + 1) * RW, :])

    def prep_wo():
        wo_t = wraw[3].T
        for i in range(NWP):
            wot[i * RW // 2:(i + 1) * RW // 2, :] = _permute_cols(wo_t[i * RW:(i + 1) * RW, :])

    def load_x(c):
        x = xin[c].astype(F32).T
        xt[c] = x
        x3 = x.reshape(D // 8, 8, TM)
        pivot = jnp.broadcast_to(x[0:1, :], (8, TM))
        d = x3 - pivot
        se[2, c] = pivot
        pacc[0, c] = jnp.sum(d, axis=0)
        pacc[1, c] = jnp.sum(d * d, axis=0)

    def colsum(p):
        return jnp.sum(p, axis=0, keepdims=True) * (1.0 / D)

    def stage_p(c, h):
        cols = slice(h * 128, (h + 1) * 128)
        load = lambda r0, r1: xt[c, r0:r1, cols]
        dm = colsum(pacc[0, c, :, cols])
        m = se[2, c, 0:1, cols] + dm
        v = jnp.maximum(colsum(pacc[1, c, :, cols]) - dm * dm, 0.0)
        mp[2 * c + h] = jnp.broadcast_to(m, (8, 128))
        r = lax.rsqrt(v + EPS)
        mr = m * r
        for j in range(NT):
            y = (load(j * 128, (j + 1) * 128) * r - mr).astype(BF16)
            xn[c, h * 64:(h + 1) * 64, j * 128:(j + 1) * 128] = pltpu.bitcast(y.T, U32)

    def store_qkv(c, t, piece):
        kind, j = divmod(t, NT)
        if kind == 0:
            qb[j, c * TM:(c + 1) * TM, :] = piece
        else:
            (kb if kind == 1 else vb)[j, HALO + c * TM:HALO + (c + 1) * TM, :] = piece

    def stage_q(c, t0, t1):
        res = jnp.dot(pltpu.bitcast(xn[c], BF16), pltpu.bitcast(wqkv[:, t0 * 128:t1 * 128], BF16),
                      preferred_element_type=F32)
        for t in range(t0, t1):
            store_qkv(c, t, res[:, (t - t0) * 128:(t - t0 + 1) * 128])

    def stage_s1(r0):
        parts = []
        for r in range(r0, r0 + RB, RG):
            q = [qb[j, r:r + RG, :] for j in range(NT)]
            for w in range(W):
                o = HALO - DIL * w + r
                acc = q[0] * kb[0, o:o + RG, :]
                for j in range(1, NT):
                    acc = acc + q[j] * kb[j, o:o + RG, :]
                parts.append(acc)
        return jnp.concatenate(parts, axis=0).astype(BF16)

    def stage_s3(r0, lg):
        res = []
        for gi, r in enumerate(range(r0, r0 + RB, RG)):
            s = [lg[(gi * W + w) * RG:(gi * W + w + 1) * RG] for w in range(W)]
            if r < HALO:
                row = r + lax.broadcasted_iota(I32, (RG, 128), 0)
                s = [s[0]] + [jnp.where(row >= DIL * w, s[w], -1e30) for w in range(1, W)]
            m = s[0]
            for w in range(1, W):
                m = jnp.maximum(m, s[w])
            e = [jnp.exp2((s[w] - m) * EXP2_SCALE) for w in range(W)]
            l = e[0]
            for w in range(1, W):
                l = l + e[w]
            inv = pl.reciprocal(l, approx=True)
            inv = inv * (2.0 - l * inv)
            outs = []
            for j in range(NT):
                acc = e[0] * vb[j, HALO + r:HALO + r + RG, :]
                for w in range(1, W):
                    o = HALO - DIL * w + r
                    acc = acc + e[w] * vb[j, o:o + RG, :]
                outs.append(acc * inv)
            res.append(jnp.concatenate(outs, axis=1))
        obuf[r0 // 2:(r0 + RB) // 2, :] = pltpu.bitcast(jnp.concatenate(res, axis=0).astype(BF16), U32)

    def stage_o(n, h):
        lhs = pltpu.bitcast(wot[h * (D // 4):(h + 1) * (D // 4), :], BF16)
        o = pltpu.bitcast(obuf[n * 64:(n + 1) * 64, :], BF16)
        return lax.dot_general(lhs, o, (((1,), (1,)), ((), ())), preferred_element_type=F32)

    def stage_res(n, h, res):
        c, hh = divmod(n, TM // 128)
        rows = slice(h * (D // 2), (h + 1) * (D // 2))
        cols = slice(hh * 128, (hh + 1) * 128)
        xnew = xt[c, rows, cols] + res
        xt[c, rows, cols] = xnew
        d = xnew.reshape(D // 16, 8, 128) - mp[n]
        return jnp.sum(d, axis=0), jnp.sum(d * d, axis=0)

    def stage_e(n, s1, s2):
        c, hh = divmod(n, TM // 128)
        cols = slice(hh * 128, (hh + 1) * 128)
        dm = colsum(s1)
        m = mp[n, 0:1, :] + dm
        v = jnp.maximum(colsum(s2) - dm * dm, 0.0)
        r1 = lax.rsqrt(v + EPS)
        r = r1 * lax.rsqrt(v * r1 * r1 + EPS)
        se[0, c, :, cols] = jnp.broadcast_to(r, (8, 128))
        se[1, c, :, cols] = jnp.broadcast_to(m * r, (8, 128))
        se[2, c, :, cols] = jnp.broadcast_to(m, (8, 128))

    def phase_a(first):
        li = lax.broadcasted_iota(I32, (128, 128), 0) >> 2
        lj = lax.broadcasted_iota(I32, (128, 128), 1) >> 2
        rsum = (li == lj).astype(BF16)
        if first:
            cp_x[0].wait()
            load_x(0)
            for h in range(2):
                stage_p(0, h)
            def q0_part(i):
                return jnp.dot(pltpu.bitcast(xn[0, :, i * qp:(i + 1) * qp], BF16),
                               pltpu.bitcast(wqkv[i * qp // 2:(i + 1) * qp // 2, 0:D], BF16),
                               preferred_element_type=F32)
            acc = None
            for i in range(NQP):
                cp_wq[i].wait()
                if i > 0:
                    part = q0_part(i - 1)
                    acc = part if acc is None else acc + part
                prep_w(0, 2 * i, 2 * i + 2)
            cp_x[1].wait()
            acc = acc + q0_part(NQP - 1)
            load_x(1)
            for h in range(2):
                stage_p(1, h)
            for j in range(NT):
                store_qkv(0, j, acc[:, j * 128:(j + 1) * 128])
            cp_x[2].wait()
            stage_q(1, 0, NT)
            load_x(2)
            for h in range(2):
                stage_p(2, h)
            cp_wk.wait()
            stage_q(2, 0, NT)
            prep_w(1)
            cp_wv.wait()
            stage_q(0, NT, 2 * NT)
            prep_w(2)
            stage_q(0, 2 * NT, 3 * NT)
        else:
            for c in range(2):
                for h in range(2):
                    stage_p(c, h)
            stage_q(0, 0, 3 * NT)

        seq = []
        nq_slots = (NCH - 1) * SPC
        for s in range(nq_slots):
            c, i = divmod(s, SPC)
            if first and c + 1 <= 2:
                t0, n0, n1 = NT + 4 * i, 2, 2
            else:
                t0, n0, n1 = 6 * i, 4, 2
            seq.append(('q', c + 1, t0, t0 + n0))
            if s >= OLAG:
                seq.append(('o',) + divmod(s - OLAG, 2))
            seq.append(('q', c + 1, t0 + n0, t0 + n0 + n1))
            if s >= LAG:
                seq.append(('r', s - LAG))
        r_next = nq_slots - LAG
        o_next = nq_slots - OLAG
        while o_next < S // 64:
            seq.append(('o',) + divmod(o_next, 2))
            o_next += 1
            if r_next < NSLOT:
                seq.append(('r', r_next))
                r_next += 1

        logits, sums = {}, {}
        done_p = {0, 1, 2} if first else {0, 1}
        done_x = {0, 1, 2}
        done_s3 = set()
        nq_seen = 0
        for op in seq:
            if op[0] == 'q':
                if first and nq_seen == 2:
                    cp_wo.wait()
                    for cc in range(3, NCH):
                        cp_x[cc].wait()
                    for cp in (cp_w1, cp_w2, cp_b1, cp_b2):
                        cp.start()
                    prep_wo()
                nq_seen += 1
                _, c, t0, t1 = op
                for cc in (c, c + 1):
                    if cc < NCH and cc not in done_p:
                        if first and cc not in done_x:
                            load_x(cc)
                            done_x.add(cc)
                        for h in range(2):
                            stage_p(cc, h)
                        done_p.add(cc)
                stage_q(c, t0, t1)
            elif op[0] == 'r':
                b = op[1]
                logits[b] = jnp.dot(stage_s1(b * RB), rsum, preferred_element_type=F32)
            else:
                _, n, h = op
                for b in (2 * n, 2 * n + 1):
                    if b not in done_s3:
                        stage_s3(b * RB, logits.pop(b))
                        done_s3.add(b)
                sums[(n, h)] = stage_res(n, h, stage_o(n, h))
                if h == 1:
                    a, b = sums.pop((n, 0)), sums.pop((n, 1))
                    stage_e(n, a[0] + b[0], a[1] + b[1])

    def phase_b(last):
        b1 = b1_ref[...]
        b2 = b2_ref[...]

        if not last:
            pacc[...] = jnp.zeros(pacc.shape, F32)

        def body(m, carry):
            rows = pl.ds(pl.multiple_of(m * TB, TB), TB)
            lhs = jnp.concatenate(
                [(xt[c, rows, :].reshape(TB // 8, 8, TM) * se[0, c] - se[1, c]).reshape(TB, TM).astype(BF16)
                 for c in range(NCH)], axis=1)
            u = jnp.dot(lhs, w1[...], preferred_element_type=F32) + b1
            u = 0.5 * u * (1.0 + jnp.tanh(GELU_C * (u + 0.044715 * (u * u * u))))
            y = jnp.dot(u.astype(BF16), w2[...], preferred_element_type=F32) + b2
            for c in range(NCH):
                xnew = xt[c, rows, :] + y[:, c * TM:(c + 1) * TM]
                if not last:
                    xt[c, rows, :] = xnew
                    d = xnew.reshape(TB // 8, 8, TM) - se[2, c]
                    pacc[0, c] = pacc[0, c] + jnp.sum(d, axis=0)
                    pacc[1, c] = pacc[1, c] + jnp.sum(d * d, axis=0)
                else:
                    stage[m, c * TM:(c + 1) * TM, :] = xnew.astype(BF16).T
                    if c % 2 == 1:
                        pltpu.make_async_copy(
                            stage.at[m, pl.ds((c - 1) * TM, 2 * TM), :],
                            out_hbm.at[pl.ds((c - 1) * TM, 2 * TM), rows],
                            sem_out.at[m * NOP + c // 2]).start()
            return carry
        lax.fori_loop(0, NB, body, 0)

    phase_a(True)
    cp_w1.wait()
    cp_w2.wait()
    cp_b1.wait()
    cp_b2.wait()
    b1_ref[...] = b1_raw[...].astype(F32).reshape(1, F)
    b2_ref[...] = b2_raw[...].astype(F32).reshape(1, S)
    phase_b(False)
    phase_a(False)
    phase_b(True)
    for m in range(NB):
        for k in range(NOP):
            pltpu.make_async_copy(stage.at[m, pl.ds(k * 2 * TM, 2 * TM), :],
                                  out_hbm.at[pl.ds(k * 2 * TM, 2 * TM), pl.ds(m * TB, TB)],
                                  sem_out.at[m * NOP + k]).wait()


@jax.jit
def pallas_interleave_layers__sliding_local_dilated__mixer_token_mlp__prompt_kernel(
    A_x: jax.Array,
    A_wqkv: jax.Array,
    A_wo: jax.Array,
    B_x: jax.Array,
    B_w1: jax.Array,
    B_b1: jax.Array,
    B_w2: jax.Array,
    B_b2: jax.Array,
):
    del B_x
    scratch = [
        pltpu.VMEM((F,), BF16),
        pltpu.VMEM((S,), BF16),
        pltpu.VMEM((1, F), F32),
        pltpu.VMEM((1, S), F32),
        pltpu.VMEM((NCH, D, TM), F32),
        pltpu.VMEM((S // 128, 8, 128), F32),
        pltpu.VMEM((3, NCH, 8, TM), F32),
        pltpu.VMEM((2, NCH, 8, TM), F32),
        pltpu.VMEM((4, D, D), BF16),
        pltpu.VMEM((D // 2, 3 * D), U32),
        pltpu.VMEM((D // 2, D), U32),
        pltpu.VMEM((S, F), BF16),
        pltpu.VMEM((F, S), BF16),
        pltpu.VMEM((NCH, TM, D), BF16),
        pltpu.VMEM((NCH, TM // 2, D), U32),
        pltpu.VMEM((NT, S, 128), F32),
        pltpu.VMEM((NT, HALO + S, 128), F32),
        pltpu.VMEM((NT, HALO + S, 128), F32),
        pltpu.VMEM((S // 2, D), U32),
        pltpu.VMEM((NB, S, TB), BF16),
        pltpu.SemaphoreType.DMA((NCH + NQP + 7,)),
        pltpu.SemaphoreType.DMA((NB * NOP,)),
    ]
    out = pl.pallas_call(
        _kernel,
        out_shape=jax.ShapeDtypeStruct((S, D), BF16),
        in_specs=[pl.BlockSpec(memory_space=pl.ANY)] * 7,
        out_specs=pl.BlockSpec(memory_space=pl.ANY),
        scratch_shapes=scratch,
        compiler_params=pltpu.CompilerParams(vmem_limit_bytes=124 * 1024 * 1024),
    )(A_x.reshape(S, D), A_wqkv, A_wo, B_w1, B_b1, B_w2, B_b2)
    return out.reshape(1, S, D)
```

```python
import math

import jax
import jax.numpy as jnp
from jax import lax
import jax.experimental.pallas as pl
import jax.experimental.pallas.tpu as pltpu

S = 2048
D = 1024
F = 3584
H = 32
DH = D // H
W = 8
DIL = 2
HALO = 16
EPS = 1e-5
TM = 256
NCH = S // TM
TB = 128
NB = D // TB
NT = D // 128
RG = 8
RB = 64
NSLOT = S // RB
SPC = TM // RB
LAG = 2
OLAG = 3 + LAG
NQP = 8
NWP = 8
RW = D // NWP
BF16 = jnp.bfloat16
F32 = jnp.float32
U32 = jnp.uint32
I32 = jnp.int32
EXP2_SCALE = (DH ** -0.5) * math.log2(math.e)
GELU_C = math.sqrt(2.0 / math.pi)


def _permute_cols(w):
    u = pltpu.bitcast(w, U32)
    tiles = [u[:, j * 128:(j + 1) * 128] for j in range(NT)]
    lane = lax.broadcasted_iota(I32, tiles[0].shape, 1)
    for tb, lb in ((2, 4), (1, 3), (0, 2)):
        keep = ((lane >> lb) & 1) == 0
        new = list(tiles)
        for j in range(NT):
            if (j >> tb) & 1:
                continue
            a, b = tiles[j], tiles[j | (1 << tb)]
            new[j] = jnp.where(keep, a, pltpu.roll(b, 1 << lb, 1))
            new[j | (1 << tb)] = jnp.where(keep, pltpu.roll(a, 128 - (1 << lb), 1), b)
        tiles = new
    return jnp.concatenate(tiles, axis=1)


def _kernel(x_hbm, wqkv_hbm, wo_hbm, w1_hbm, b1_hbm, w2_hbm, b2_hbm, out_hbm,
            b1_raw, b2_raw, b1_ref, b2_ref, xt, mp, se, pacc, wraw, wqkv, wot, w1, w2, xin, xn,
            qb, kb, vb, obuf, stage, sem_in, sem_out):
    cp_x = [pltpu.make_async_copy(x_hbm.at[pl.ds(c * TM, TM), :], xin.at[c], sem_in.at[c])
            for c in range(NCH)]
    qp = D // NQP
    cp_wq = [pltpu.make_async_copy(wqkv_hbm.at[pl.ds(i * qp, qp), pl.ds(0, D)],
                                   wraw.at[0, pl.ds(i * qp, qp), :], sem_in.at[NCH + i])
             for i in range(NQP)]
    sb = NCH + NQP
    cp_wk = pltpu.make_async_copy(wqkv_hbm.at[:, pl.ds(D, D)], wraw.at[1], sem_in.at[sb])
    cp_wv = pltpu.make_async_copy(wqkv_hbm.at[:, pl.ds(2 * D, D)], wraw.at[2], sem_in.at[sb + 1])
    cp_wo = pltpu.make_async_copy(wo_hbm, wraw.at[3], sem_in.at[sb + 2])
    cp_w1 = pltpu.make_async_copy(w1_hbm, w1, sem_in.at[sb + 3])
    cp_w2 = pltpu.make_async_copy(w2_hbm, w2, sem_in.at[sb + 4])
    cp_b1 = pltpu.make_async_copy(b1_hbm, b1_raw, sem_in.at[sb + 5])
    cp_b2 = pltpu.make_async_copy(b2_hbm, b2_raw, sem_in.at[sb + 6])
    for cp in (cp_x[0], *cp_wq, cp_x[1], cp_x[2], cp_wk, cp_wv, cp_wo, *cp_x[3:]):
        cp.start()
    for b in (kb, vb):
        b[:, 0:HALO, :] = jnp.zeros((NT, HALO, 128), F32)

    def prep_w(t, i0=0, i1=NWP):
        for i in range(i0, i1):
            wqkv[i * RW // 2:(i + 1) * RW // 2, t * D:(t + 1) * D] = _permute_cols(wraw[t, i * RW:(i + 1) * RW, :])

    def prep_wo():
        wo_t = wraw[3].T
        for i in range(NWP):
            wot[i * RW // 2:(i + 1) * RW // 2, :] = _permute_cols(wo_t[i * RW:(i + 1) * RW, :])

    def load_x(c):
        x = xin[c].astype(F32).T
        xt[c] = x
        x3 = x.reshape(D // 8, 8, TM)
        pivot = jnp.broadcast_to(x[0:1, :], (8, TM))
        d = x3 - pivot
        se[2, c] = pivot
        pacc[0, c] = jnp.sum(d, axis=0)
        pacc[1, c] = jnp.sum(d * d, axis=0)

    def colsum(p):
        return jnp.sum(p, axis=0, keepdims=True) * (1.0 / D)

    def stage_p(c, h):
        cols = slice(h * 128, (h + 1) * 128)
        load = lambda r0, r1: xt[c, r0:r1, cols]
        dm = colsum(pacc[0, c, :, cols])
        m = se[2, c, 0:1, cols] + dm
        v = jnp.maximum(colsum(pacc[1, c, :, cols]) - dm * dm, 0.0)
        mp[2 * c + h] = jnp.broadcast_to(m, (8, 128))
        r = lax.rsqrt(v + EPS)
        mr = m * r
        for j in range(NT):
            y = (load(j * 128, (j + 1) * 128) * r - mr).astype(BF16)
            xn[c, h * 64:(h + 1) * 64, j * 128:(j + 1) * 128] = pltpu.bitcast(y.T, U32)

    def store_qkv(c, t, piece):
        kind, j = divmod(t, NT)
        if kind == 0:
            qb[j, c * TM:(c + 1) * TM, :] = piece
        else:
            (kb if kind == 1 else vb)[j, HALO + c * TM:HALO + (c + 1) * TM, :] = piece

    def stage_q(c, t0, t1):
        res = jnp.dot(pltpu.bitcast(xn[c], BF16), pltpu.bitcast(wqkv[:, t0 * 128:t1 * 128], BF16),
                      preferred_element_type=F32)
        for t in range(t0, t1):
            store_qkv(c, t, res[:, (t - t0) * 128:(t - t0 + 1) * 128])

    def stage_s1(r0):
        parts = []
        for r in range(r0, r0 + RB, RG):
            q = [qb[j, r:r + RG, :] for j in range(NT)]
            for w in range(W):
                o = HALO - DIL * w + r
                acc = q[0] * kb[0, o:o + RG, :]
                for j in range(1, NT):
                    acc = acc + q[j] * kb[j, o:o + RG, :]
                parts.append(acc)
        return jnp.concatenate(parts, axis=0).astype(BF16)

    def stage_s3(r0, lg):
        res = []
        for gi, r in enumerate(range(r0, r0 + RB, RG)):
            s = [lg[(gi * W + w) * RG:(gi * W + w + 1) * RG] for w in range(W)]
            if r < HALO:
                row = r + lax.broadcasted_iota(I32, (RG, 128), 0)
                s = [s[0]] + [jnp.where(row >= DIL * w, s[w], -1e30) for w in range(1, W)]
            m = s[0]
            for w in range(1, W):
                m = jnp.maximum(m, s[w])
            e = [jnp.exp2((s[w] - m) * EXP2_SCALE) for w in range(W)]
            l = e[0]
            for w in range(1, W):
                l = l + e[w]
            inv = pl.reciprocal(l, approx=True)
            inv = inv * (2.0 - l * inv)
            outs = []
            for j in range(NT):
                acc = e[0] * vb[j, HALO + r:HALO + r + RG, :]
                for w in range(1, W):
                    o = HALO - DIL * w + r
                    acc = acc + e[w] * vb[j, o:o + RG, :]
                outs.append(acc * inv)
            res.append(jnp.concatenate(outs, axis=1))
        obuf[r0 // 2:(r0 + RB) // 2, :] = pltpu.bitcast(jnp.concatenate(res, axis=0).astype(BF16), U32)

    def stage_o(n, h):
        lhs = pltpu.bitcast(wot[h * (D // 4):(h + 1) * (D // 4), :], BF16)
        o = pltpu.bitcast(obuf[n * 64:(n + 1) * 64, :], BF16)
        return lax.dot_general(lhs, o, (((1,), (1,)), ((), ())), preferred_element_type=F32)

    def stage_res(n, h, res):
        c, hh = divmod(n, TM // 128)
        rows = slice(h * (D // 2), (h + 1) * (D // 2))
        cols = slice(hh * 128, (hh + 1) * 128)
        xnew = xt[c, rows, cols] + res
        xt[c, rows, cols] = xnew
        d = xnew.reshape(D // 16, 8, 128) - mp[n]
        return jnp.sum(d, axis=0), jnp.sum(d * d, axis=0)

    def stage_e(n, s1, s2):
        c, hh = divmod(n, TM // 128)
        cols = slice(hh * 128, (hh + 1) * 128)
        dm = colsum(s1)
        m = mp[n, 0:1, :] + dm
        v = jnp.maximum(colsum(s2) - dm * dm, 0.0)
        r1 = lax.rsqrt(v + EPS)
        r = r1 * lax.rsqrt(v * r1 * r1 + EPS)
        se[0, c, :, cols] = jnp.broadcast_to(r, (8, 128))
        se[1, c, :, cols] = jnp.broadcast_to(m * r, (8, 128))
        se[2, c, :, cols] = jnp.broadcast_to(m, (8, 128))

    def phase_a(first):
        li = lax.broadcasted_iota(I32, (128, 128), 0) >> 2
        lj = lax.broadcasted_iota(I32, (128, 128), 1) >> 2
        rsum = (li == lj).astype(BF16)
        if first:
            cp_x[0].wait()
            load_x(0)
            for h in range(2):
                stage_p(0, h)

            def q0_part(i):
                return jnp.dot(pltpu.bitcast(xn[0, :, i * qp:(i + 1) * qp], BF16),
                               pltpu.bitcast(wqkv[i * qp // 2:(i + 1) * qp // 2, 0:D], BF16),
                               preferred_element_type=F32)
            acc = None
            for i in range(NQP):
                cp_wq[i].wait()
                if i > 0:
                    part = q0_part(i - 1)
                    acc = part if acc is None else acc + part
                prep_w(0, i * NWP // NQP, (i + 1) * NWP // NQP)
            cp_x[1].wait()
            acc = acc + q0_part(NQP - 1)
            load_x(1)
            for h in range(2):
                stage_p(1, h)
            for j in range(NT):
                store_qkv(0, j, acc[:, j * 128:(j + 1) * 128])
            cp_x[2].wait()
            stage_q(1, 0, NT)
            load_x(2)
            for h in range(2):
                stage_p(2, h)
            cp_wk.wait()
            stage_q(2, 0, NT)
            prep_w(1)
            cp_wv.wait()
            stage_q(0, NT, 2 * NT)
            prep_w(2)
            stage_q(0, 2 * NT, 3 * NT)
        else:
            for c in range(2):
                for h in range(2):
                    stage_p(c, h)
            stage_q(0, 0, 3 * NT)

        seq = []
        nq_slots = (NCH - 1) * SPC
        for s in range(nq_slots):
            c, i = divmod(s, SPC)
            if first and c + 1 <= 2:
                t0, n0, n1 = NT + 4 * i, 2, 2
            else:
                t0, n0, n1 = 6 * i, 4, 2
            seq.append(('q', c + 1, t0, t0 + n0))
            if s >= OLAG:
                seq.append(('o',) + divmod(s - OLAG, 2))
            seq.append(('q', c + 1, t0 + n0, t0 + n0 + n1))
            if s >= LAG:
                seq.append(('r', s - LAG))
        r_next = nq_slots - LAG
        o_next = nq_slots - OLAG
        while o_next < S // 64:
            seq.append(('o',) + divmod(o_next, 2))
            o_next += 1
            if r_next < NSLOT:
                seq.append(('r', r_next))
                r_next += 1

        logits, sums = {}, {}
        done_p = {0, 1, 2} if first else {0, 1}
        done_x = {0, 1, 2}
        done_s3 = set()
        nq_seen = 0
        for op in seq:
            if op[0] == 'q':
                if first and nq_seen == 2:
                    cp_wo.wait()
                    for cc in range(3, NCH):
                        cp_x[cc].wait()
                    for cp in (cp_w1, cp_w2, cp_b1, cp_b2):
                        cp.start()
                    prep_wo()
                nq_seen += 1
                _, c, t0, t1 = op
                for cc in (c, c + 1):
                    if cc < NCH and cc not in done_p:
                        if first and cc not in done_x:
                            load_x(cc)
                            done_x.add(cc)
                        for h in range(2):
                            stage_p(cc, h)
                        done_p.add(cc)
                stage_q(c, t0, t1)
            elif op[0] == 'r':
                b = op[1]
                logits[b] = jnp.dot(stage_s1(b * RB), rsum, preferred_element_type=F32)
            else:
                _, n, h = op
                for b in (2 * n, 2 * n + 1):
                    if b not in done_s3:
                        stage_s3(b * RB, logits.pop(b))
                        done_s3.add(b)
                sums[(n, h)] = stage_res(n, h, stage_o(n, h))
                if h == 1:
                    a, b = sums.pop((n, 0)), sums.pop((n, 1))
                    stage_e(n, a[0] + b[0], a[1] + b[1])

    def phase_b(last):
        b1 = b1_ref[...]
        b2 = b2_ref[...]

        if not last:
            pacc[...] = jnp.zeros(pacc.shape, F32)

        def body(m, carry):
            rows = pl.ds(pl.multiple_of(m * TB, TB), TB)
            lhs = jnp.concatenate(
                [(xt[c, rows, :].reshape(TB // 8, 8, TM) * se[0, c] - se[1, c]).reshape(TB, TM).astype(BF16)
                 for c in range(NCH)], axis=1)
            u = jnp.dot(lhs, w1[...], preferred_element_type=F32) + b1
            u = 0.5 * u * (1.0 + jnp.tanh(GELU_C * (u + 0.044715 * (u * u * u))))
            y = jnp.dot(u.astype(BF16), w2[...], preferred_element_type=F32) + b2
            for c in range(NCH):
                xnew = xt[c, rows, :] + y[:, c * TM:(c + 1) * TM]
                if not last:
                    xt[c, rows, :] = xnew
                    d = xnew.reshape(TB // 8, 8, TM) - se[2, c]
                    pacc[0, c] = pacc[0, c] + jnp.sum(d, axis=0)
                    pacc[1, c] = pacc[1, c] + jnp.sum(d * d, axis=0)
                else:
                    stage[m, c * TM:(c + 1) * TM, :] = xnew.astype(BF16).T
                    pltpu.make_async_copy(stage.at[m, pl.ds(c * TM, TM), :],
                                          out_hbm.at[pl.ds(c * TM, TM), rows], sem_out.at[0]).start()
            return carry
        lax.fori_loop(0, NB, body, 0)

    phase_a(True)
    cp_w1.wait()
    cp_w2.wait()
    cp_b1.wait()
    cp_b2.wait()
    b1_ref[...] = b1_raw[...].astype(F32).reshape(1, F)
    b2_ref[...] = b2_raw[...].astype(F32).reshape(1, S)
    phase_b(False)
    phase_a(False)
    phase_b(True)
    pltpu.make_async_copy(stage, stage, sem_out.at[0]).wait()


@jax.jit
def pallas_interleave_layers__sliding_local_dilated__mixer_token_mlp__prompt_kernel(
    A_x: jax.Array,
    A_wqkv: jax.Array,
    A_wo: jax.Array,
    B_x: jax.Array,
    B_w1: jax.Array,
    B_b1: jax.Array,
    B_w2: jax.Array,
    B_b2: jax.Array,
):
    del B_x
    scratch = [
        pltpu.VMEM((F,), BF16),
        pltpu.VMEM((S,), BF16),
        pltpu.VMEM((1, F), F32),
        pltpu.VMEM((1, S), F32),
        pltpu.VMEM((NCH, D, TM), F32),
        pltpu.VMEM((S // 128, 8, 128), F32),
        pltpu.VMEM((3, NCH, 8, TM), F32),
        pltpu.VMEM((2, NCH, 8, TM), F32),
        pltpu.VMEM((4, D, D), BF16),
        pltpu.VMEM((D // 2, 3 * D), U32),
        pltpu.VMEM((D // 2, D), U32),
        pltpu.VMEM((S, F), BF16),
        pltpu.VMEM((F, S), BF16),
        pltpu.VMEM((NCH, TM, D), BF16),
        pltpu.VMEM((NCH, TM // 2, D), U32),
        pltpu.VMEM((NT, S, 128), F32),
        pltpu.VMEM((NT, HALO + S, 128), F32),
        pltpu.VMEM((NT, HALO + S, 128), F32),
        pltpu.VMEM((S // 2, D), U32),
        pltpu.VMEM((NB, S, TB), BF16),
        pltpu.SemaphoreType.DMA((NCH + NQP + 7,)),
        pltpu.SemaphoreType.DMA((1,)),
    ]
    out = pl.pallas_call(
        _kernel,
        out_shape=jax.ShapeDtypeStruct((S, D), BF16),
        in_specs=[pl.BlockSpec(memory_space=pl.ANY)] * 7,
        out_specs=pl.BlockSpec(memory_space=pl.ANY),
        scratch_shapes=scratch,
        compiler_params=pltpu.CompilerParams(vmem_limit_bytes=124 * 1024 * 1024),
    )(A_x.reshape(S, D), A_wqkv, A_wo, B_w1, B_b1, B_w2, B_b2)
    return out.reshape(1, S, D)
```

```python
import math

import jax
import jax.numpy as jnp
from jax import lax
import jax.experimental.pallas as pl
import jax.experimental.pallas.tpu as pltpu

S = 2048
D = 1024
F = 3584
H = 32
DH = D // H
W = 8
DIL = 2
HALO = 16
EPS = 1e-5
TM = 256
NCH = S // TM
TB = 128
NB = D // TB
NT = D // 128
RG = 8
RB = 64
NSLOT = S // RB
SPC = TM // RB
LAG = 2
OLAG = 3 + LAG
OM = 128
NQP = 8
NWP = 8
RW = D // NWP
BF16 = jnp.bfloat16
F32 = jnp.float32
U32 = jnp.uint32
I32 = jnp.int32
EXP2_SCALE = (DH ** -0.5) * math.log2(math.e)
GELU_C = math.sqrt(2.0 / math.pi)


def _permute_cols(w):
    u = pltpu.bitcast(w, U32)
    tiles = [u[:, j * 128:(j + 1) * 128] for j in range(NT)]
    lane = lax.broadcasted_iota(I32, tiles[0].shape, 1)
    for tb, lb in ((2, 4), (1, 3), (0, 2)):
        keep = ((lane >> lb) & 1) == 0
        new = list(tiles)
        for j in range(NT):
            if (j >> tb) & 1:
                continue
            a, b = tiles[j], tiles[j | (1 << tb)]
            new[j] = jnp.where(keep, a, pltpu.roll(b, 1 << lb, 1))
            new[j | (1 << tb)] = jnp.where(keep, pltpu.roll(a, 128 - (1 << lb), 1), b)
        tiles = new
    return jnp.concatenate(tiles, axis=1)


def _kernel(x_hbm, wqkv_hbm, wo_hbm, w1_hbm, b1_hbm, w2_hbm, b2_hbm, out_hbm,
            b1_raw, b2_raw, b1_ref, b2_ref, xt, mp, se, pacc, wraw, wqkv, wot, w1, w2, xin, xn,
            qb, kb, vb, obuf, stage, sem_in, sem_out):
    cp_x = [pltpu.make_async_copy(x_hbm.at[pl.ds(c * TM, TM), :], xin.at[c], sem_in.at[c])
            for c in range(NCH)]
    qp = D // NQP
    cp_wq = [pltpu.make_async_copy(wqkv_hbm.at[pl.ds(i * qp, qp), pl.ds(0, D)],
                                   wraw.at[0, pl.ds(i * qp, qp), :], sem_in.at[NCH + i])
             for i in range(NQP)]
    sb = NCH + NQP
    cp_wk = pltpu.make_async_copy(wqkv_hbm.at[:, pl.ds(D, D)], wraw.at[1], sem_in.at[sb])
    cp_wv = pltpu.make_async_copy(wqkv_hbm.at[:, pl.ds(2 * D, D)], wraw.at[2], sem_in.at[sb + 1])
    cp_wo = pltpu.make_async_copy(wo_hbm, wraw.at[3], sem_in.at[sb + 2])
    cp_w1 = pltpu.make_async_copy(w1_hbm, w1, sem_in.at[sb + 3])
    cp_w2 = pltpu.make_async_copy(w2_hbm, w2, sem_in.at[sb + 4])
    cp_b1 = pltpu.make_async_copy(b1_hbm, b1_raw, sem_in.at[sb + 5])
    cp_b2 = pltpu.make_async_copy(b2_hbm, b2_raw, sem_in.at[sb + 6])
    for cp in (cp_x[0], *cp_wq, cp_x[1], cp_x[2], cp_wk, cp_wv, cp_wo, *cp_x[3:]):
        cp.start()
    for b in (kb, vb):
        b[:, 0:HALO, :] = jnp.zeros((NT, HALO, 128), F32)

    def prep_w(t, i0=0, i1=NWP):
        for i in range(i0, i1):
            wqkv[i * RW // 2:(i + 1) * RW // 2, t * D:(t + 1) * D] = _permute_cols(wraw[t, i * RW:(i + 1) * RW, :])

    def prep_wo():
        wo_t = wraw[3].T
        for i in range(NWP):
            wot[i * RW // 2:(i + 1) * RW // 2, :] = _permute_cols(wo_t[i * RW:(i + 1) * RW, :])

    def load_x(c):
        x = xin[c].astype(F32).T
        xt[c] = x
        x3 = x.reshape(D // 8, 8, TM)
        pivot = jnp.broadcast_to(x[0:1, :], (8, TM))
        d = x3 - pivot
        se[2, c] = pivot
        pacc[0, c] = jnp.sum(d, axis=0)
        pacc[1, c] = jnp.sum(d * d, axis=0)

    def colsum(p):
        return jnp.sum(p, axis=0, keepdims=True) * (1.0 / D)

    def stage_p(c, h):
        cols = slice(h * 128, (h + 1) * 128)
        load = lambda r0, r1: xt[c, r0:r1, cols]
        dm = colsum(pacc[0, c, :, cols])
        m = se[2, c, 0:1, cols] + dm
        v = jnp.maximum(colsum(pacc[1, c, :, cols]) - dm * dm, 0.0)
        mp[2 * c + h] = jnp.broadcast_to(m, (8, 128))
        r = lax.rsqrt(v + EPS)
        mr = m * r
        for j in range(NT):
            y = (load(j * 128, (j + 1) * 128) * r - mr).astype(BF16)
            xn[c, h * 64:(h + 1) * 64, j * 128:(j + 1) * 128] = pltpu.bitcast(y.T, U32)

    def store_qkv(c, t, piece):
        kind, j = divmod(t, NT)
        if kind == 0:
            qb[j, c * TM:(c + 1) * TM, :] = piece
        else:
            (kb if kind == 1 else vb)[j, HALO + c * TM:HALO + (c + 1) * TM, :] = piece

    def stage_q(c, t0, t1):
        res = jnp.dot(pltpu.bitcast(xn[c], BF16), pltpu.bitcast(wqkv[:, t0 * 128:t1 * 128], BF16),
                      preferred_element_type=F32)
        for t in range(t0, t1):
            store_qkv(c, t, res[:, (t - t0) * 128:(t - t0 + 1) * 128])

    def stage_s1(r0):
        parts = []
        for r in range(r0, r0 + RB, RG):
            q = [qb[j, r:r + RG, :] for j in range(NT)]
            for w in range(W):
                o = HALO - DIL * w + r
                acc = q[0] * kb[0, o:o + RG, :]
                for j in range(1, NT):
                    acc = acc + q[j] * kb[j, o:o + RG, :]
                parts.append(acc)
        return jnp.concatenate(parts, axis=0).astype(BF16)

    def stage_s3(r0, lg):
        res = []
        for gi, r in enumerate(range(r0, r0 + RB, RG)):
            s = [lg[(gi * W + w) * RG:(gi * W + w + 1) * RG] for w in range(W)]
            if r < HALO:
                row = r + lax.broadcasted_iota(I32, (RG, 128), 0)
                s = [s[0]] + [jnp.where(row >= DIL * w, s[w], -1e30) for w in range(1, W)]
            m = s[0]
            for w in range(1, W):
                m = jnp.maximum(m, s[w])
            e = [jnp.exp2((s[w] - m) * EXP2_SCALE) for w in range(W)]
            l = e[0]
            for w in range(1, W):
                l = l + e[w]
            inv = pl.reciprocal(l, approx=True)
            inv = inv * (2.0 - l * inv)
            outs = []
            for j in range(NT):
                acc = e[0] * vb[j, HALO + r:HALO + r + RG, :]
                for w in range(1, W):
                    o = HALO - DIL * w + r
                    acc = acc + e[w] * vb[j, o:o + RG, :]
                outs.append(acc * inv)
            res.append(jnp.concatenate(outs, axis=1))
        obuf[r0 // 2:(r0 + RB) // 2, :] = pltpu.bitcast(jnp.concatenate(res, axis=0).astype(BF16), U32)

    def stage_o(n, h):
        o = pltpu.bitcast(obuf[n * 64:(n + 1) * 64, :], BF16)
        outs = []
        for k in range(D // 2 // OM):
            r0 = (h * (D // 2) + k * OM) // 2
            lhs = pltpu.bitcast(wot[r0:r0 + OM // 2, :], BF16)
            outs.append(lax.dot_general(lhs, o, (((1,), (1,)), ((), ())), preferred_element_type=F32))
        return jnp.concatenate(outs, axis=0)

    def stage_res(n, h, res):
        c, hh = divmod(n, TM // 128)
        rows = slice(h * (D // 2), (h + 1) * (D // 2))
        cols = slice(hh * 128, (hh + 1) * 128)
        xnew = xt[c, rows, cols] + res
        xt[c, rows, cols] = xnew
        d = xnew.reshape(D // 16, 8, 128) - mp[n]
        return jnp.sum(d, axis=0), jnp.sum(d * d, axis=0)

    def stage_e(n, s1, s2):
        c, hh = divmod(n, TM // 128)
        cols = slice(hh * 128, (hh + 1) * 128)
        dm = colsum(s1)
        m = mp[n, 0:1, :] + dm
        v = jnp.maximum(colsum(s2) - dm * dm, 0.0)
        r1 = lax.rsqrt(v + EPS)
        r = r1 * lax.rsqrt(v * r1 * r1 + EPS)
        se[0, c, :, cols] = jnp.broadcast_to(r, (8, 128))
        se[1, c, :, cols] = jnp.broadcast_to(m * r, (8, 128))
        se[2, c, :, cols] = jnp.broadcast_to(m, (8, 128))

    def phase_a(first):
        li = lax.broadcasted_iota(I32, (128, 128), 0) >> 2
        lj = lax.broadcasted_iota(I32, (128, 128), 1) >> 2
        rsum = (li == lj).astype(BF16)
        if first:
            cp_x[0].wait()
            load_x(0)
            for h in range(2):
                stage_p(0, h)

            def q0_part(i):
                return jnp.dot(pltpu.bitcast(xn[0, :, i * qp:(i + 1) * qp], BF16),
                               pltpu.bitcast(wqkv[i * qp // 2:(i + 1) * qp // 2, 0:D], BF16),
                               preferred_element_type=F32)
            acc = None
            for i in range(NQP):
                cp_wq[i].wait()
                if i > 0:
                    part = q0_part(i - 1)
                    acc = part if acc is None else acc + part
                prep_w(0, i * NWP // NQP, (i + 1) * NWP // NQP)
            cp_x[1].wait()
            acc = acc + q0_part(NQP - 1)
            load_x(1)
            for h in range(2):
                stage_p(1, h)
            for j in range(NT):
                store_qkv(0, j, acc[:, j * 128:(j + 1) * 128])
            cp_x[2].wait()
            stage_q(1, 0, NT)
            load_x(2)
            for h in range(2):
                stage_p(2, h)
            cp_wk.wait()
            stage_q(2, 0, NT)
            prep_w(1)
            cp_wv.wait()
            stage_q(0, NT, 2 * NT)
            prep_w(2)
            stage_q(0, 2 * NT, 3 * NT)
        else:
            for c in range(2):
                for h in range(2):
                    stage_p(c, h)
            stage_q(0, 0, 3 * NT)

        seq = []
        nq_slots = (NCH - 1) * SPC
        for s in range(nq_slots):
            c, i = divmod(s, SPC)
            if first and c + 1 <= 2:
                t0, n0, n1 = NT + 4 * i, 2, 2
            else:
                t0, n0, n1 = 6 * i, 4, 2
            seq.append(('q', c + 1, t0, t0 + n0))
            if s >= OLAG:
                seq.append(('o',) + divmod(s - OLAG, 2))
            seq.append(('q', c + 1, t0 + n0, t0 + n0 + n1))
            if s >= LAG:
                seq.append(('r', s - LAG))
        r_next = nq_slots - LAG
        o_next = nq_slots - OLAG
        while o_next < S // 64:
            seq.append(('o',) + divmod(o_next, 2))
            o_next += 1
            if r_next < NSLOT:
                seq.append(('r', r_next))
                r_next += 1

        logits, sums = {}, {}
        done_p = {0, 1, 2} if first else {0, 1}
        done_x = {0, 1, 2}
        done_s3 = set()
        nq_seen = 0
        for op in seq:
            if op[0] == 'q':
                if first and nq_seen == 2:
                    cp_wo.wait()
                    for cc in range(3, NCH):
                        cp_x[cc].wait()
                    for cp in (cp_w1, cp_w2, cp_b1, cp_b2):
                        cp.start()
                    prep_wo()
                nq_seen += 1
                _, c, t0, t1 = op
                for cc in (c, c + 1):
                    if cc < NCH and cc not in done_p:
                        if first and cc not in done_x:
                            load_x(cc)
                            done_x.add(cc)
                        for h in range(2):
                            stage_p(cc, h)
                        done_p.add(cc)
                stage_q(c, t0, t1)
            elif op[0] == 'r':
                b = op[1]
                logits[b] = jnp.dot(stage_s1(b * RB), rsum, preferred_element_type=F32)
            else:
                _, n, h = op
                for b in (2 * n, 2 * n + 1):
                    if b not in done_s3:
                        stage_s3(b * RB, logits.pop(b))
                        done_s3.add(b)
                sums[(n, h)] = stage_res(n, h, stage_o(n, h))
                if h == 1:
                    a, b = sums.pop((n, 0)), sums.pop((n, 1))
                    stage_e(n, a[0] + b[0], a[1] + b[1])

    def phase_b(last):
        b1 = b1_ref[...]
        b2 = b2_ref[...]

        if not last:
            pacc[...] = jnp.zeros(pacc.shape, F32)

        def body(m, carry):
            rows = pl.ds(pl.multiple_of(m * TB, TB), TB)
            lhs = jnp.concatenate(
                [(xt[c, rows, :].reshape(TB // 8, 8, TM) * se[0, c] - se[1, c]).reshape(TB, TM).astype(BF16)
                 for c in range(NCH)], axis=1)
            u = jnp.dot(lhs, w1[...], preferred_element_type=F32) + b1
            u = 0.5 * u * (1.0 + jnp.tanh(GELU_C * (u + 0.044715 * (u * u * u))))
            y = jnp.dot(u.astype(BF16), w2[...], preferred_element_type=F32) + b2
            for c in range(NCH):
                xnew = xt[c, rows, :] + y[:, c * TM:(c + 1) * TM]
                if not last:
                    xt[c, rows, :] = xnew
                    d = xnew.reshape(TB // 8, 8, TM) - se[2, c]
                    pacc[0, c] = pacc[0, c] + jnp.sum(d, axis=0)
                    pacc[1, c] = pacc[1, c] + jnp.sum(d * d, axis=0)
                else:
                    stage[m, c * TM:(c + 1) * TM, :] = xnew.astype(BF16).T
                    pltpu.make_async_copy(stage.at[m, pl.ds(c * TM, TM), :],
                                          out_hbm.at[pl.ds(c * TM, TM), rows], sem_out.at[0]).start()
            return carry
        lax.fori_loop(0, NB, body, 0)

    phase_a(True)
    cp_w1.wait()
    cp_w2.wait()
    cp_b1.wait()
    cp_b2.wait()
    b1_ref[...] = b1_raw[...].astype(F32).reshape(1, F)
    b2_ref[...] = b2_raw[...].astype(F32).reshape(1, S)
    phase_b(False)
    phase_a(False)
    phase_b(True)
    pltpu.make_async_copy(stage, stage, sem_out.at[0]).wait()


@jax.jit
def pallas_interleave_layers__sliding_local_dilated__mixer_token_mlp__prompt_kernel(
    A_x: jax.Array,
    A_wqkv: jax.Array,
    A_wo: jax.Array,
    B_x: jax.Array,
    B_w1: jax.Array,
    B_b1: jax.Array,
    B_w2: jax.Array,
    B_b2: jax.Array,
):
    del B_x
    scratch = [
        pltpu.VMEM((F,), BF16),
        pltpu.VMEM((S,), BF16),
        pltpu.VMEM((1, F), F32),
        pltpu.VMEM((1, S), F32),
        pltpu.VMEM((NCH, D, TM), F32),
        pltpu.VMEM((S // 128, 8, 128), F32),
        pltpu.VMEM((3, NCH, 8, TM), F32),
        pltpu.VMEM((2, NCH, 8, TM), F32),
        pltpu.VMEM((4, D, D), BF16),
        pltpu.VMEM((D // 2, 3 * D), U32),
        pltpu.VMEM((D // 2, D), U32),
        pltpu.VMEM((S, F), BF16),
        pltpu.VMEM((F, S), BF16),
        pltpu.VMEM((NCH, TM, D), BF16),
        pltpu.VMEM((NCH, TM // 2, D), U32),
        pltpu.VMEM((NT, S, 128), F32),
        pltpu.VMEM((NT, HALO + S, 128), F32),
        pltpu.VMEM((NT, HALO + S, 128), F32),
        pltpu.VMEM((S // 2, D), U32),
        pltpu.VMEM((NB, S, TB), BF16),
        pltpu.SemaphoreType.DMA((NCH + NQP + 7,)),
        pltpu.SemaphoreType.DMA((1,)),
    ]
    out = pl.pallas_call(
        _kernel,
        out_shape=jax.ShapeDtypeStruct((S, D), BF16),
        in_specs=[pl.BlockSpec(memory_space=pl.ANY)] * 7,
        out_specs=pl.BlockSpec(memory_space=pl.ANY),
        scratch_shapes=scratch,
        compiler_params=pltpu.CompilerParams(vmem_limit_bytes=124 * 1024 * 1024),
    )(A_x.reshape(S, D), A_wqkv, A_wo, B_w1, B_b1, B_w2, B_b2)
    return out.reshape(1, S, D)
```

```python
import math

import jax
import jax.numpy as jnp
from jax import lax
import jax.experimental.pallas as pl
import jax.experimental.pallas.tpu as pltpu

S = 2048
D = 1024
F = 3584
H = 32
DH = D // H
W = 8
DIL = 2
HALO = 16
EPS = 1e-5
TM = 256
NCH = S // TM
TB = 128
NB = D // TB
NT = D // 128
RG = 8
RB = 64
NSLOT = S // RB
SPC = TM // RB
LAG = 2
OLAG = 3 + LAG
OM = 128
NQP = 8
NWP = 8
RW = D // NWP
OUT_GROUPS = {2: 0, 5: 3, 6: 6, 7: 7}
BF16 = jnp.bfloat16
F32 = jnp.float32
U32 = jnp.uint32
I32 = jnp.int32
EXP2_SCALE = (DH ** -0.5) * math.log2(math.e)
GELU_C = math.sqrt(2.0 / math.pi)


def _permute_cols(w):
    u = pltpu.bitcast(w, U32)
    tiles = [u[:, j * 128:(j + 1) * 128] for j in range(NT)]
    lane = lax.broadcasted_iota(I32, tiles[0].shape, 1)
    for tb, lb in ((2, 4), (1, 3), (0, 2)):
        keep = ((lane >> lb) & 1) == 0
        new = list(tiles)
        for j in range(NT):
            if (j >> tb) & 1:
                continue
            a, b = tiles[j], tiles[j | (1 << tb)]
            new[j] = jnp.where(keep, a, pltpu.roll(b, 1 << lb, 1))
            new[j | (1 << tb)] = jnp.where(keep, pltpu.roll(a, 128 - (1 << lb), 1), b)
        tiles = new
    return jnp.concatenate(tiles, axis=1)


def _kernel(x_hbm, wqkv_hbm, wo_hbm, w1_hbm, b1_hbm, w2_hbm, b2_hbm, out_hbm,
            b1_raw, b2_raw, b1_ref, b2_ref, xt, mp, se, pacc, wraw, wqkv, wot, w1, w2, xin, xn,
            qb, kb, vb, obuf, stage, sem_in, sem_out):
    cp_x = [pltpu.make_async_copy(x_hbm.at[pl.ds(c * TM, TM), :], xin.at[c], sem_in.at[c])
            for c in range(NCH)]
    qp = D // NQP
    cp_wq = [pltpu.make_async_copy(wqkv_hbm.at[pl.ds(i * qp, qp), pl.ds(0, D)],
                                   wraw.at[0, pl.ds(i * qp, qp), :], sem_in.at[NCH + i])
             for i in range(NQP)]
    sb = NCH + NQP
    cp_wk = pltpu.make_async_copy(wqkv_hbm.at[:, pl.ds(D, D)], wraw.at[1], sem_in.at[sb])
    cp_wv = pltpu.make_async_copy(wqkv_hbm.at[:, pl.ds(2 * D, D)], wraw.at[2], sem_in.at[sb + 1])
    cp_wo = pltpu.make_async_copy(wo_hbm, wraw.at[3], sem_in.at[sb + 2])
    cp_w1 = pltpu.make_async_copy(w1_hbm, w1, sem_in.at[sb + 3])
    cp_w2 = pltpu.make_async_copy(w2_hbm, w2, sem_in.at[sb + 4])
    cp_b1 = pltpu.make_async_copy(b1_hbm, b1_raw, sem_in.at[sb + 5])
    cp_b2 = pltpu.make_async_copy(b2_hbm, b2_raw, sem_in.at[sb + 6])
    for cp in (cp_x[0], *cp_wq, cp_x[1], cp_x[2], cp_wk, cp_wv, cp_wo, *cp_x[3:]):
        cp.start()
    for b in (kb, vb):
        b[:, 0:HALO, :] = jnp.zeros((NT, HALO, 128), F32)

    def prep_w(t, i0=0, i1=NWP):
        for i in range(i0, i1):
            wqkv[i * RW // 2:(i + 1) * RW // 2, t * D:(t + 1) * D] = _permute_cols(wraw[t, i * RW:(i + 1) * RW, :])

    def prep_wo():
        wo_t = wraw[3].T
        for i in range(NWP):
            wot[i * RW // 2:(i + 1) * RW // 2, :] = _permute_cols(wo_t[i * RW:(i + 1) * RW, :])

    def load_x(c):
        x = xin[c].astype(F32).T
        xt[c] = x
        x3 = x.reshape(D // 8, 8, TM)
        pivot = jnp.broadcast_to(x[0:1, :], (8, TM))
        d = x3 - pivot
        se[2, c] = pivot
        pacc[0, c] = jnp.sum(d, axis=0)
        pacc[1, c] = jnp.sum(d * d, axis=0)

    def colsum(p):
        return jnp.sum(p, axis=0, keepdims=True) * (1.0 / D)

    def stage_p(c, h):
        cols = slice(h * 128, (h + 1) * 128)
        load = lambda r0, r1: xt[c, r0:r1, cols]
        dm = colsum(pacc[0, c, :, cols])
        m = se[2, c, 0:1, cols] + dm
        v = jnp.maximum(colsum(pacc[1, c, :, cols]) - dm * dm, 0.0)
        mp[2 * c + h] = jnp.broadcast_to(m, (8, 128))
        r = lax.rsqrt(v + EPS)
        mr = m * r
        for j in range(NT):
            y = (load(j * 128, (j + 1) * 128) * r - mr).astype(BF16)
            xn[c, h * 64:(h + 1) * 64, j * 128:(j + 1) * 128] = pltpu.bitcast(y.T, U32)

    def store_qkv(c, t, piece):
        kind, j = divmod(t, NT)
        if kind == 0:
            qb[j, c * TM:(c + 1) * TM, :] = piece
        else:
            (kb if kind == 1 else vb)[j, HALO + c * TM:HALO + (c + 1) * TM, :] = piece

    def stage_q(c, t0, t1):
        res = jnp.dot(pltpu.bitcast(xn[c], BF16), pltpu.bitcast(wqkv[:, t0 * 128:t1 * 128], BF16),
                      preferred_element_type=F32)
        for t in range(t0, t1):
            store_qkv(c, t, res[:, (t - t0) * 128:(t - t0 + 1) * 128])

    def stage_s1(r0):
        parts = []
        for r in range(r0, r0 + RB, RG):
            q = [qb[j, r:r + RG, :] for j in range(NT)]
            for w in range(W):
                o = HALO - DIL * w + r
                acc = q[0] * kb[0, o:o + RG, :]
                for j in range(1, NT):
                    acc = acc + q[j] * kb[j, o:o + RG, :]
                parts.append(acc)
        return jnp.concatenate(parts, axis=0).astype(BF16)

    def stage_s3(r0, lg):
        res = []
        for gi, r in enumerate(range(r0, r0 + RB, RG)):
            s = [lg[(gi * W + w) * RG:(gi * W + w + 1) * RG] for w in range(W)]
            if r < HALO:
                row = r + lax.broadcasted_iota(I32, (RG, 128), 0)
                s = [s[0]] + [jnp.where(row >= DIL * w, s[w], -1e30) for w in range(1, W)]
            m = s[0]
            for w in range(1, W):
                m = jnp.maximum(m, s[w])
            e = [jnp.exp2((s[w] - m) * EXP2_SCALE) for w in range(W)]
            l = e[0]
            for w in range(1, W):
                l = l + e[w]
            inv = pl.reciprocal(l, approx=True)
            inv = inv * (2.0 - l * inv)
            outs = []
            for j in range(NT):
                acc = e[0] * vb[j, HALO + r:HALO + r + RG, :]
                for w in range(1, W):
                    o = HALO - DIL * w + r
                    acc = acc + e[w] * vb[j, o:o + RG, :]
                outs.append(acc * inv)
            res.append(jnp.concatenate(outs, axis=1))
        obuf[r0 // 2:(r0 + RB) // 2, :] = pltpu.bitcast(jnp.concatenate(res, axis=0).astype(BF16), U32)

    def stage_o(n, h):
        o = pltpu.bitcast(obuf[n * 64:(n + 1) * 64, :], BF16)
        outs = []
        for k in range(D // 2 // OM):
            r0 = (h * (D // 2) + k * OM) // 2
            lhs = pltpu.bitcast(wot[r0:r0 + OM // 2, :], BF16)
            outs.append(lax.dot_general(lhs, o, (((1,), (1,)), ((), ())), preferred_element_type=F32))
        return jnp.concatenate(outs, axis=0)

    def stage_res(n, h, res):
        c, hh = divmod(n, TM // 128)
        rows = slice(h * (D // 2), (h + 1) * (D // 2))
        cols = slice(hh * 128, (hh + 1) * 128)
        xnew = xt[c, rows, cols] + res
        xt[c, rows, cols] = xnew
        d = xnew.reshape(D // 16, 8, 128) - mp[n]
        return jnp.sum(d, axis=0), jnp.sum(d * d, axis=0)

    def stage_e(n, s1, s2):
        c, hh = divmod(n, TM // 128)
        cols = slice(hh * 128, (hh + 1) * 128)
        dm = colsum(s1)
        m = mp[n, 0:1, :] + dm
        v = jnp.maximum(colsum(s2) - dm * dm, 0.0)
        r1 = lax.rsqrt(v + EPS)
        r = r1 * lax.rsqrt(v * r1 * r1 + EPS)
        se[0, c, :, cols] = jnp.broadcast_to(r, (8, 128))
        se[1, c, :, cols] = jnp.broadcast_to(m * r, (8, 128))
        se[2, c, :, cols] = jnp.broadcast_to(m, (8, 128))

    def phase_a(first):
        li = lax.broadcasted_iota(I32, (128, 128), 0) >> 2
        lj = lax.broadcasted_iota(I32, (128, 128), 1) >> 2
        rsum = (li == lj).astype(BF16)
        if first:
            cp_x[0].wait()
            load_x(0)
            for h in range(2):
                stage_p(0, h)

            def q0_part(i):
                return jnp.dot(pltpu.bitcast(xn[0, :, i * qp:(i + 1) * qp], BF16),
                               pltpu.bitcast(wqkv[i * qp // 2:(i + 1) * qp // 2, 0:D], BF16),
                               preferred_element_type=F32)
            acc = None
            for i in range(NQP):
                cp_wq[i].wait()
                if i > 0:
                    part = q0_part(i - 1)
                    acc = part if acc is None else acc + part
                prep_w(0, i * NWP // NQP, (i + 1) * NWP // NQP)
            cp_x[1].wait()
            acc = acc + q0_part(NQP - 1)
            load_x(1)
            for h in range(2):
                stage_p(1, h)
            for j in range(NT):
                store_qkv(0, j, acc[:, j * 128:(j + 1) * 128])
            cp_x[2].wait()
            stage_q(1, 0, NT)
            load_x(2)
            for h in range(2):
                stage_p(2, h)
            cp_wk.wait()
            stage_q(2, 0, NT)
            prep_w(1)
            cp_wv.wait()
            stage_q(0, NT, 2 * NT)
            prep_w(2)
            stage_q(0, 2 * NT, 3 * NT)
        else:
            for c in range(2):
                for h in range(2):
                    stage_p(c, h)
            stage_q(0, 0, 3 * NT)

        seq = []
        nq_slots = (NCH - 1) * SPC
        for s in range(nq_slots):
            c, i = divmod(s, SPC)
            if first and c + 1 <= 2:
                t0, n0, n1 = NT + 4 * i, 2, 2
            else:
                t0, n0, n1 = 6 * i, 4, 2
            seq.append(('q', c + 1, t0, t0 + n0))
            if s >= OLAG:
                seq.append(('o',) + divmod(s - OLAG, 2))
            seq.append(('q', c + 1, t0 + n0, t0 + n0 + n1))
            if s >= LAG:
                seq.append(('r', s - LAG))
        r_next = nq_slots - LAG
        o_next = nq_slots - OLAG
        while o_next < S // 64:
            seq.append(('o',) + divmod(o_next, 2))
            o_next += 1
            if r_next < NSLOT:
                seq.append(('r', r_next))
                r_next += 1

        logits, sums = {}, {}
        done_p = {0, 1, 2} if first else {0, 1}
        done_x = {0, 1, 2}
        done_s3 = set()
        nq_seen = 0
        for op in seq:
            if op[0] == 'q':
                if first and nq_seen == 2:
                    cp_wo.wait()
                    for cc in range(3, NCH):
                        cp_x[cc].wait()
                    for cp in (cp_w1, cp_w2, cp_b1, cp_b2):
                        cp.start()
                    prep_wo()
                nq_seen += 1
                _, c, t0, t1 = op
                for cc in (c, c + 1):
                    if cc < NCH and cc not in done_p:
                        if first and cc not in done_x:
                            load_x(cc)
                            done_x.add(cc)
                        for h in range(2):
                            stage_p(cc, h)
                        done_p.add(cc)
                stage_q(c, t0, t1)
            elif op[0] == 'r':
                b = op[1]
                logits[b] = jnp.dot(stage_s1(b * RB), rsum, preferred_element_type=F32)
            else:
                _, n, h = op
                for b in (2 * n, 2 * n + 1):
                    if b not in done_s3:
                        stage_s3(b * RB, logits.pop(b))
                        done_s3.add(b)
                sums[(n, h)] = stage_res(n, h, stage_o(n, h))
                if h == 1:
                    a, b = sums.pop((n, 0)), sums.pop((n, 1))
                    stage_e(n, a[0] + b[0], a[1] + b[1])

    def phase_b(last):
        b1 = b1_ref[...]
        b2 = b2_ref[...]

        if not last:
            pacc[...] = jnp.zeros(pacc.shape, F32)

        def body(m, carry):
            rows = pl.ds(pl.multiple_of(m * TB, TB), TB)
            lhs = jnp.concatenate(
                [(xt[c, rows, :].reshape(TB // 8, 8, TM) * se[0, c] - se[1, c]).reshape(TB, TM).astype(BF16)
                 for c in range(NCH)], axis=1)
            u = jnp.dot(lhs, w1[...], preferred_element_type=F32) + b1
            u = 0.5 * u * (1.0 + jnp.tanh(GELU_C * (u + 0.044715 * (u * u * u))))
            y = jnp.dot(u.astype(BF16), w2[...], preferred_element_type=F32) + b2
            for c in range(NCH):
                xnew = xt[c, rows, :] + y[:, c * TM:(c + 1) * TM]
                if not last:
                    xt[c, rows, :] = xnew
                    d = xnew.reshape(TB // 8, 8, TM) - se[2, c]
                    pacc[0, c] = pacc[0, c] + jnp.sum(d, axis=0)
                    pacc[1, c] = pacc[1, c] + jnp.sum(d * d, axis=0)
                else:
                    stage[m, c * TM:(c + 1) * TM, :] = xnew.astype(BF16).T
                    if c in OUT_GROUPS:
                        c0 = OUT_GROUPS[c]
                        pltpu.make_async_copy(stage.at[m, pl.ds(c0 * TM, (c + 1 - c0) * TM), :],
                                              out_hbm.at[pl.ds(c0 * TM, (c + 1 - c0) * TM), rows],
                                              sem_out.at[0]).start()
            return carry
        lax.fori_loop(0, NB, body, 0)

    phase_a(True)
    cp_w1.wait()
    cp_w2.wait()
    cp_b1.wait()
    cp_b2.wait()
    b1_ref[...] = b1_raw[...].astype(F32).reshape(1, F)
    b2_ref[...] = b2_raw[...].astype(F32).reshape(1, S)
    phase_b(False)
    phase_a(False)
    phase_b(True)
    pltpu.make_async_copy(stage, stage, sem_out.at[0]).wait()


@jax.jit
def pallas_interleave_layers__sliding_local_dilated__mixer_token_mlp__prompt_kernel(
    A_x: jax.Array,
    A_wqkv: jax.Array,
    A_wo: jax.Array,
    B_x: jax.Array,
    B_w1: jax.Array,
    B_b1: jax.Array,
    B_w2: jax.Array,
    B_b2: jax.Array,
):
    del B_x
    scratch = [
        pltpu.VMEM((F,), BF16),
        pltpu.VMEM((S,), BF16),
        pltpu.VMEM((1, F), F32),
        pltpu.VMEM((1, S), F32),
        pltpu.VMEM((NCH, D, TM), F32),
        pltpu.VMEM((S // 128, 8, 128), F32),
        pltpu.VMEM((3, NCH, 8, TM), F32),
        pltpu.VMEM((2, NCH, 8, TM), F32),
        pltpu.VMEM((4, D, D), BF16),
        pltpu.VMEM((D // 2, 3 * D), U32),
        pltpu.VMEM((D // 2, D), U32),
        pltpu.VMEM((S, F), BF16),
        pltpu.VMEM((F, S), BF16),
        pltpu.VMEM((NCH, TM, D), BF16),
        pltpu.VMEM((NCH, TM // 2, D), U32),
        pltpu.VMEM((NT, S, 128), F32),
        pltpu.VMEM((NT, HALO + S, 128), F32),
        pltpu.VMEM((NT, HALO + S, 128), F32),
        pltpu.VMEM((S // 2, D), U32),
        pltpu.VMEM((NB, S, TB), BF16),
        pltpu.SemaphoreType.DMA((NCH + NQP + 7,)),
        pltpu.SemaphoreType.DMA((1,)),
    ]
    out = pl.pallas_call(
        _kernel,
        out_shape=jax.ShapeDtypeStruct((S, D), BF16),
        in_specs=[pl.BlockSpec(memory_space=pl.ANY)] * 7,
        out_specs=pl.BlockSpec(memory_space=pl.ANY),
        scratch_shapes=scratch,
        compiler_params=pltpu.CompilerParams(vmem_limit_bytes=124 * 1024 * 1024),
    )(A_x.reshape(S, D), A_wqkv, A_wo, B_w1, B_b1, B_w2, B_b2)
    return out.reshape(1, S, D)
```
